```python
import jax
import jax.numpy as jnp

def _softmax(x, axis=-1):
    return jax.nn.softmax(x, axis=axis)

def _gelu(x):
    return jax.nn.gelu(x, approximate=True)

def _silu(x):
    return jax.nn.silu(x)

def _sigmoid(x):
    return jax.nn.sigmoid(x)

def _layernorm(x, axis=-1, eps=1e-05):
    m = jnp.mean(x, axis=axis, keepdims=True)
    v = jnp.var(x, axis=axis, keepdims=True)
    return (x - m) / jnp.sqrt(v + eps)

def _scatter_add(tgt, idx, src, axis=0):
    return tgt.at[idx].add(src)

def _segment_sum(src, seg, n):
    return jax.ops.segment_sum(src, seg, n)

class _Rng:

    def __init__(self, key):
        self._k = key

    def _next(self):
        self._k, sub = jax.random.split(self._k)
        return sub

    def normal(self, shape):
        return jax.random.normal(self._next(), shape, dtype=jnp.bfloat16)

    def randint(self, lo, hi, shape):
        return jax.random.randint(self._next(), shape, lo, hi, dtype=jnp.int32)

    def uniform(self, shape, lo=0.0, hi=1.0):
        return jax.random.uniform(self._next(), shape, jnp.bfloat16, lo, hi)

    def permutation(self, n):
        return jax.random.permutation(self._next(), n)
kernel_name = 'interleave_layers__memory_aug_infini_attn__moe_arch_mod__prompt'

def setup_inputs():
    _rng = _Rng(jax.random.key(int.from_bytes(__import__("os").urandom(4), "little")))
    _w = lambda a: (lambda t: t.astype(jnp.bfloat16) if jnp.issubdtype(t.dtype, jnp.floating) else t)(jnp.asarray(a))

    def _A_setup():
        B, S, D, H = (1, 2048, 1024, 32)
        N = 4
        L = max(1, S // N)
        sc = D ** (-0.5)
        return {'x': _w((lambda *s: _rng.normal(s) * 0.05)(B, N * L, D)), 'wq': _w((lambda *s: _rng.normal(s) * 0.05)(D, D) * sc), 'wk': _w((lambda *s: _rng.normal(s) * 0.05)(D, D) * sc), 'wv': _w((lambda *s: _rng.normal(s) * 0.05)(D, D) * sc), 'wo': _w((lambda *s: _rng.normal(s) * 0.05)(D, D) * sc), 'beta': _w((lambda *s: _rng.normal(s) * 0.05)(H))}
    _A_in = _A_setup()

    def _B_setup():
        B, S, D, F, C = (1, 2048, 1024, 3584, 2)
        return {'x': _w((lambda *s: _rng.normal(s) * 0.05)(B, S, D)), 'w_r': _w((lambda *s: _rng.normal(s) * 0.05)(D)), 'w_gate': _w((lambda *s: _rng.normal(s) * 0.05)(D, F)), 'w_up': _w((lambda *s: _rng.normal(s) * 0.05)(D, F)), 'w_down': _w((lambda *s: _rng.normal(s) * 0.05)(F, D))}
    _B_in = _B_setup()
    return {'A_x': _A_in['x'], 'A_wq': _A_in['wq'], 'A_wk': _A_in['wk'], 'A_wv': _A_in['wv'], 'A_wo': _A_in['wo'], 'A_beta': _A_in['beta'], 'B_x': _B_in['x'], 'B_w_r': _B_in['w_r'], 'B_w_gate': _B_in['w_gate'], 'B_w_up': _B_in['w_up'], 'B_w_down': _B_in['w_down']}

def reference(A_x, A_wq, A_wk, A_wv, A_wo, A_beta, B_x, B_w_r, B_w_gate, B_w_up, B_w_down):

    def _A_ref(x, wq, wk, wv, wo, beta):
        B, S, D = x.shape
        H = 32
        Dh = D // H
        N = 4
        L = S // N
        q = (lambda x, *d: x.transpose(*d))((x @ wq).reshape(B, S, H, Dh), 0, 2, 1, 3).reshape(B, H, N, L, Dh)
        k = (lambda x, *d: x.transpose(*d))((x @ wk).reshape(B, S, H, Dh), 0, 2, 1, 3).reshape(B, H, N, L, Dh)
        v = (lambda x, *d: x.transpose(*d))((x @ wv).reshape(B, S, H, Dh), 0, 2, 1, 3).reshape(B, H, N, L, Dh)
        phi = lambda t: jnp.where(t > 0, t + 1.0, jnp.exp(t))
        scale = Dh ** (-0.5)
        ar = jnp.arange(L)
        mask = (lambda x, dt: x.astype(dt))(ar[:, None] < ar[None, :], x.dtype) * -1000000000.0
        g = _sigmoid(beta).reshape(1, H, 1, 1)
        M = jnp.einsum('bhd,bhe->bhde', q[:, :, 0, 0, :] * 0.0, q[:, :, 0, 0, :] * 0.0)
        z = q[:, :, 0, 0, :] * 0.0
        outs = []
        for s in range(N):
            qs, ks, vs = (q[:, :, s].copy(), k[:, :, s].copy(), v[:, :, s].copy())
            logits = jnp.einsum('bhqd,bhkd->bhqk', qs, ks) * scale + mask
            p = _softmax(logits, axis=-1)
            a_dot = jnp.einsum('bhqk,bhkd->bhqd', p, vs)
            pq = phi(qs)
            num = jnp.einsum('bhld,bhde->bhle', pq, M)
            den = jnp.einsum('bhld,bhd->bhl', pq, z)[..., None] + 1e-06
            a_mem = num / den
            o = g * a_mem + (1.0 - g) * a_dot
            outs.append(o)
            pk = phi(ks)
            M = M + jnp.einsum('bhld,bhle->bhde', pk, vs)
            z = z + jnp.einsum('bhld->bhd', pk)
        o = (lambda x, *d: x.transpose(*d))(jnp.stack(outs, 2).reshape(B, H, S, Dh), 0, 2, 1, 3).reshape(B, S, D)
        return o @ wo

    def _B_ref(x, w_r, w_gate, w_up, w_down):
        B, S, D = x.shape
        C = 2
        r = x @ w_r
        idx = jnp.argsort(-r, axis=-1)[:, :C]
        idx_e = jnp.repeat(idx.reshape(B, C, 1), D, axis=2)
        x_sel = jnp.take_along_axis(x, idx_e, axis=1)
        g = _silu(x_sel @ w_gate)
        u = x_sel @ w_up
        y = g * u @ w_down
        r_sel = _sigmoid(jnp.take_along_axis(r, idx, axis=1))
        y = y * r_sel.reshape(B, C, 1)
        b_off = (jnp.arange(B) * S).reshape(B, 1)
        flat_idx = (idx + b_off).reshape(B * C)
        zero = (x * 0.0).reshape(B * S, D)
        upd = _scatter_add(zero, flat_idx, y.reshape(B * C, D), axis=0)
        return x + upd.reshape(B, S, D)
    x = A_x
    x = x + _A_ref(_layernorm(x, axis=-1), A_wq, A_wk, A_wv, A_wo, A_beta)
    x = x + _B_ref(_layernorm(x, axis=-1), B_w_r, B_w_gate, B_w_up, B_w_down)
    x = x + _A_ref(_layernorm(x, axis=-1), A_wq, A_wk, A_wv, A_wo, A_beta)
    x = x + _B_ref(_layernorm(x, axis=-1), B_w_r, B_w_gate, B_w_up, B_w_down)
    return x
```

```python
import jax
import jax.numpy as jnp
import numpy as np
from jax import lax
import jax.experimental.pallas as pl
import jax.experimental.pallas.tpu as pltpu

S, D, F = 2048, 1024, 3584
H, DH = 32, 32
NSEG, L = 4, 512
G, T = 8, 128
NT = L // T
OFF = (0, 128, 384, 768)
NEG = -1e30
QSCALE = float(DH ** -0.5 * np.log2(np.e))
BF = jnp.bfloat16
F32 = jnp.float32


def dot_nt(a, b):
    return lax.dot_general(a, b, (((1,), (1,)), ((), ())), preferred_element_type=F32)


def dot_nn(a, b):
    return lax.dot_general(a, b, (((1,), (0,)), ((), ())), preferred_element_type=F32)


def rb(x):
    return x.astype(BF).astype(F32)


def layernorm(x):
    m = jnp.mean(x, axis=-1, keepdims=True)
    c = x - m
    v = jnp.mean(c * c, axis=-1, keepdims=True)
    s = rb(jnp.sqrt(rb(rb(v) + 1e-5)))
    d = rb(x - rb(m))
    return (d * (1.0 / s)).astype(BF)


def phi(t):
    return jnp.where(t > 0, t + 1.0, jnp.exp(t))


def head_mask(x, h):
    u = pltpu.bitcast(x, jnp.uint32)
    lane = lax.broadcasted_iota(jnp.int32, u.shape, 1)
    u = jnp.where((lane >= DH * h) & (lane < DH * h + DH), u, jnp.uint32(0))
    return pltpu.bitcast(u, BF)


def kernel(x_hbm, wq_hbm, wk_hbm, wv_hbm, wo_hbm, beta_ref, wr_ref, wg_hbm, wu_hbm, wd_hbm,
           out_hbm,
           X, XM, XN2, XN, WQ, WK, WV, WVT, WO, WG, WU, WD,
           QS, KK, PQ, PK, VT, SB, MB, OT, OB, MT, ZZ, AMEM, GATE, RALL, sems):
    cps = dict(
        x=pltpu.make_async_copy(x_hbm, X, sems.at[0]),
        wq=pltpu.make_async_copy(wq_hbm, WQ, sems.at[1]),
        wk=pltpu.make_async_copy(wk_hbm, WK, sems.at[2]),
        wv=pltpu.make_async_copy(wv_hbm, WV, sems.at[3]),
        wo=pltpu.make_async_copy(wo_hbm, WO, sems.at[4]),
        wg=pltpu.make_async_copy(wg_hbm, WG, sems.at[5]),
        wu=pltpu.make_async_copy(wu_hbm, WU, sems.at[6]),
        wd=pltpu.make_async_copy(wd_hbm, WD, sems.at[7]),
    )
    for n in ("x", "wv", "wk", "wq"):
        cps[n].start()
    gate = jax.nn.sigmoid(beta_ref[...].astype(F32))
    for j in range(H):
        GATE[j] = jnp.broadcast_to(gate[:, j:j + 1], (8, 128))
    wr8 = wr_ref[...].astype(F32)
    wr16 = jnp.concatenate(
        [jnp.broadcast_to(wr8[c:c + 1, :], (16, 128)) for c in range(8)], axis=1).astype(BF)
    cps["x"].wait()
    cps["wv"].wait()
    for n in ("wo", "wg", "wu", "wd"):
        cps[n].start()
    for i in range(D // T):
        for j in range(D // T):
            WVT[j * T:(j + 1) * T, i * T:(i + 1) * T] = (
                WV[i * T:(i + 1) * T, j * T:(j + 1) * T].astype(F32).T.astype(BF))
    cps["wk"].wait()
    cps["wq"].wait()

    rowT = lax.broadcasted_iota(jnp.int32, (T, T), 0)
    colT = lax.broadcasted_iota(jnp.int32, (T, T), 1)

    def p1(g, h, qt, slot):
        qm = head_mask(QS[g, qt * T:(qt + 1) * T, :], h)
        m = None
        for kt in range(qt + 1):
            s = dot_nt(KK[g, kt * T:(kt + 1) * T, :], qm)
            if kt == qt:
                s = jnp.where(rowT <= colT, s, NEG)
            SB[slot, OFF[qt] + kt * T:OFF[qt] + (kt + 1) * T, :] = s
            mt = jnp.max(s.reshape(16, 8, 128), axis=0)
            m = mt if m is None else jnp.maximum(m, mt)
        m = jnp.max(m, axis=0, keepdims=True)
        MB[slot, qt] = jnp.broadcast_to(m, (8, 128))

    def p2(g, h, qt, slot):
        m = MB[slot, qt]
        l = acc = None
        for kt in range(qt + 1):
            s = SB[slot, OFF[qt] + kt * T:OFF[qt] + (kt + 1) * T, :]
            p = jnp.exp2(s.reshape(16, 8, 128) - m[None])
            ps = jnp.sum(p, axis=0)
            pv = dot_nn(VT[g, DH * h:DH * h + DH, kt * T:(kt + 1) * T],
                        p.reshape(T, 128).astype(BF))
            l = ps if l is None else l + ps
            acc = pv if acc is None else acc + pv
        lt = jnp.sum(l, axis=0, keepdims=True)
        w = (1.0 - GATE[4 * g + h][0:1, :]) / lt
        OT[g, DH * h:DH * h + DH, qt * T:(qt + 1) * T] += acc * w

    def mem_part(g):
        r = dot_nt(AMEM[g], PQ[g])
        for h in range(4):
            den = r[128 + 8 * h:136 + 8 * h, :][0:1, :] + 1e-6
            OT[g, DH * h:DH * h + DH, :] = r[DH * h:DH * h + DH, :] * (GATE[4 * g + h][0:1, 0:1] / den)
        pk = PK[g]
        upd = dot_nn(VT[g], pk)
        rr = lax.broadcasted_iota(jnp.int32, (128, 128), 0) // DH
        cc = lax.broadcasted_iota(jnp.int32, (128, 128), 1) // DH
        mt = MT[g] + jnp.where(rr == cc, upd, 0.0)
        MT[g] = mt
        z = jnp.sum(pk.astype(F32).reshape(L // 8, 8, 128), axis=0)
        z = ZZ[g] + jnp.broadcast_to(jnp.sum(z, axis=0, keepdims=True), (8, 128))
        ZZ[g] = z
        AMEM[g, 0:128, :] = mt.astype(BF)
        zr = lax.broadcasted_iota(jnp.int32, (32, 128), 0) // 8
        zc = lax.broadcasted_iota(jnp.int32, (32, 128), 1) // DH
        z32 = jnp.concatenate([z, z, z, z], axis=0)
        AMEM[g, 128:160, :] = jnp.where(zr == zc, z32, 0.0).astype(BF)

    def layer(li, carry):
        MT[...] = jnp.zeros_like(MT)
        ZZ[...] = jnp.zeros_like(ZZ)
        AMEM[...] = jnp.zeros_like(AMEM)
        RALL[...] = jnp.zeros_like(RALL)

        def segment(s, c):
            r0 = pl.multiple_of(s * L, L)
            for r in range(NT):
                x = X[pl.ds(r0 + r * T, T), :].astype(F32)
                XN[r * T:(r + 1) * T, :] = layernorm(x)
            xn = XN[...]
            q = dot_nn(xn, WQ[...])
            for g in range(G):
                qg = q[:, g * 128:(g + 1) * 128]
                QS[g] = (qg * QSCALE).astype(BF)
                PQ[g] = phi(qg).astype(BF)
            k = dot_nn(xn, WK[...])
            for g in range(G):
                kg = k[:, g * 128:(g + 1) * 128]
                KK[g] = kg.astype(BF)
                PK[g] = phi(kg).astype(BF)
            vt = dot_nt(WVT[...], xn)
            for g in range(G):
                VT[g] = vt[g * 128:(g + 1) * 128, :].astype(BF)
            for qt in range(NT):
                p1(0, 0, qt, 0)

            def group(g, c2):
                gn = jnp.minimum(g + 1, G - 1)
                mem_part(g)
                for h in range(4):
                    hn = (h + 1) % 4
                    gg = g if h < 3 else gn
                    for qt in range(NT):
                        p2(g, h, qt, h % 2)
                        p1(gg, hn, qt, hn % 2)
                for qt in range(NT):
                    OB[g, qt * T:(qt + 1) * T, :] = OT[g, :, qt * T:(qt + 1) * T].T.astype(BF)
                return c2
            lax.fori_loop(0, G, group, 0)
            @pl.when(jnp.logical_and(li == 0, s == 0))
            def _():
                cps["wo"].wait()
            o = jnp.concatenate([OB[g] for g in range(G)], axis=1)
            y = dot_nn(o, WO[...])
            for r in range(NT):
                rows = pl.ds(r0 + r * T, T)
                xm = (X[rows, :].astype(F32) + rb(y[r * T:(r + 1) * T, :])).astype(BF)
                XM[rows, :] = xm
                xmf = xm.astype(F32)
                xn2 = layernorm(xmf)
                XN2[rows, :] = xn2
                X[rows, :] = (xmf + xn2.astype(F32)).astype(BF)
                rr = dot_nt(wr16, xn2)
                ri = lax.broadcasted_iota(jnp.int32, (16, 128), 0)
                RALL[...] = jnp.where(ri == s * NT + r, rr, RALL[...])
            return c
        lax.fori_loop(0, NSEG, segment, 0)

        @pl.when(li == 0)
        def _():
            cps["wg"].wait()
            cps["wu"].wait()
            cps["wd"].wait()
        rv = rb(RALL[...])
        idx = (lax.broadcasted_iota(jnp.int32, (16, 128), 0) * 128
               + lax.broadcasted_iota(jnp.int32, (16, 128), 1))
        m1 = jnp.max(rv)
        i1 = jnp.min(jnp.where(rv == m1, idx, S))
        i1 = jnp.clip(i1, 0, S - 1)
        rv2 = jnp.where(idx == i1, -jnp.inf, rv)
        m2 = jnp.max(rv2)
        i2 = jnp.min(jnp.where((rv2 == m2) & (idx != i1), idx, S))
        i2 = jnp.clip(i2, 0, S - 1)
        row16 = lax.broadcasted_iota(jnp.int32, (16, D), 0)
        sel = []
        for i in (i1, i2):
            base = pl.multiple_of((i // 16) * 16, 16)
            blk = XN2[pl.ds(base, 16), :].astype(F32)
            sel.append(jnp.sum(jnp.where(row16 == i - base, blk, 0.0), axis=0, keepdims=True))
        xs = jnp.where(row16 == 0, sel[0], jnp.where(row16 == 1, sel[1], 0.0)).astype(BF)
        gg = rb(dot_nn(xs, WG[...]))
        uu = rb(dot_nn(xs, WU[...]))
        hh = (rb(gg * jax.nn.sigmoid(gg)) * uu).astype(BF)
        yy = rb(dot_nn(hh, WD[...]))
        for j, (i, mv) in enumerate(((i1, m1), (i2, m2))):
            base = pl.multiple_of((i // 16) * 16, 16)
            rs = rb(jax.nn.sigmoid(jnp.full((1, D), mv, F32)))
            upd = rb(yy[j:j + 1, :] * rs)
            blk = XN2[pl.ds(base, 16), :].astype(F32)
            nb = jnp.where(row16 == i - base, rb(blk + upd), blk)
            XN2[pl.ds(base, 16), :] = nb.astype(BF)
            X[pl.ds(base, 16), :] = (XM[pl.ds(base, 16), :].astype(F32) + nb).astype(BF)
        return carry

    lax.fori_loop(0, 2, layer, 0)
    cp = pltpu.make_async_copy(X, out_hbm, sems.at[8])
    cp.start()
    cp.wait()


@jax.jit
def pallas_interleave_layers__memory_aug_infini_attn__moe_arch_mod__prompt_kernel(
    A_x, A_wq, A_wk, A_wv, A_wo, A_beta, B_x, B_w_r, B_w_gate, B_w_up, B_w_down):
    del B_x
    any_spec = pl.BlockSpec(memory_space=pl.ANY)
    vm = pltpu.VMEM
    blk = vm((G, L, 128), BF)
    out = pl.pallas_call(
        kernel,
        out_shape=jax.ShapeDtypeStruct((S, D), BF),
        in_specs=[any_spec, any_spec, any_spec, any_spec, any_spec,
                  pl.BlockSpec(memory_space=vm), pl.BlockSpec(memory_space=vm),
                  any_spec, any_spec, any_spec],
        out_specs=any_spec,
        scratch_shapes=[
            vm((S, D), BF), vm((S, D), BF), vm((S, D), BF), vm((L, D), BF),
            vm((D, D), BF), vm((D, D), BF), vm((D, D), BF), vm((D, D), BF), vm((D, D), BF),
            vm((D, F), BF), vm((D, F), BF), vm((F, D), BF),
            blk, blk, blk, blk, vm((G, 128, L), BF),
            vm((2, 1280, 128), F32), vm((2, NT, 8, 128), F32),
            vm((G, 128, L), F32), blk,
            vm((G, 128, 128), F32), vm((G, 8, 128), F32), vm((G, 160, 128), BF),
            vm((H, 8, 128), F32), vm((16, 128), F32),
            pltpu.SemaphoreType.DMA((9,)),
        ],
        compiler_params=pltpu.CompilerParams(vmem_limit_bytes=110 * 1024 * 1024),
        name="fused",
    )(A_x.reshape(S, D), A_wq, A_wk, A_wv, A_wo, A_beta.reshape(1, H), B_w_r.reshape(8, 128),
      B_w_gate, B_w_up, B_w_down)
    return out.reshape(1, S, D)
```

```python
import jax
import jax.numpy as jnp
import numpy as np
from jax import lax
import jax.experimental.pallas as pl
import jax.experimental.pallas.tpu as pltpu

S, D, F = 2048, 1024, 3584
H, DH = 32, 32
NSEG, L = 4, 512
G, T = 8, 128
NT = L // T
NF = F // T
OFF = (0, 128, 384, 768)
NEG = -1e30
EPS = 1e-5
QSCALE = float(DH ** -0.5 * np.log2(np.e))
BF = jnp.bfloat16
F32 = jnp.float32
import os
LNR = int(os.environ.get('LNR', '32'))
ONLY = os.environ.get('ONLY')
VAR = os.environ.get('VAR', '')
CHAIN = int(os.environ.get('CHAIN', '1'))
FLAGS = {k: True for k in os.environ.get('FLAGS', '').split(',') if k} or None


def dot_nt(a, b):
    return lax.dot_general(a, b, (((1,), (1,)), ((), ())), preferred_element_type=F32)


def dot_nn(a, b):
    return lax.dot_general(a, b, (((1,), (0,)), ((), ())), preferred_element_type=F32)


def rb(x):
    return x.astype(BF).astype(F32)


def layernorm(x, chain=None):
    m = jnp.sum(x, axis=-1, keepdims=True) * (1.0 / D)
    if chain is not None and chain.get("tok") is not None:
        m = jnp.where(chain["never"], chain["tok"], m)
    c = x - m
    v = jnp.sum(c * c, axis=-1, keepdims=True) * (1.0 / D)
    a = rb(rb(v) + EPS)
    y = lax.rsqrt(a)
    s = rb(a * y)
    y = y * (2.0 - s * y)
    if chain is not None:
        chain["tok"] = y
    return c * y


def phi(t):
    return jnp.where(t > 0, t + 1.0, jnp.exp(t))


def head_mask(x, h):
    u = pltpu.bitcast(x, jnp.uint32)
    lane = lax.broadcasted_iota(jnp.int32, u.shape, 1)
    u = jnp.where((lane >= DH * h) & (lane < DH * h + DH), u, jnp.uint32(0))
    return pltpu.bitcast(u, BF)


def interleave(main, *bgs):
    main = list(main)
    bgs = [list(b) for b in bgs]
    done = [0] * len(bgs)
    n = len(main)
    for i, piece in enumerate(main):
        piece()
        for bi, b in enumerate(bgs):
            upto = (i + 1) * len(b) // n
            while done[bi] < upto:
                b[done[bi]]()
                done[bi] += 1


def kernel(x_hbm, wq_hbm, wk_hbm, wv_hbm, wo_hbm, beta_ref, wr_ref, wg_hbm, wu_hbm, wd_hbm,
           out_hbm,
           X, XM, XN2, XN, WQ, WK, WV, WVT, WO, WG, WU, WD,
           QS, KK, PQ, PK, VT, SB, MB, OT, OB, MT, ZZ, AMEM, GATE, WR, RALL, sems):
    def cp(src, dst, i):
        return pltpu.make_async_copy(src, dst, sems.at[i])
    cx = [cp(x_hbm.at[pl.ds(s * L, L), :], X.at[pl.ds(s * L, L), :], s) for s in range(NSEG)]
    cwq, cwk, cwv, cwo = (cp(wq_hbm, WQ, 4), cp(wk_hbm, WK, 5), cp(wv_hbm, WV, 6), cp(wo_hbm, WO, 7))
    cwg = [cp(wg_hbm.at[:, pl.ds(j * T, T)], WG.at[j], 8) for j in range(NF)]
    cwu = [cp(wu_hbm.at[:, pl.ds(j * T, T)], WU.at[j], 8) for j in range(NF)]
    cwd = [cp(wd_hbm.at[:, pl.ds(j * T, T)], WD.at[j], 8) for j in range(D // T)]
    cout = [cp(X.at[pl.ds(s * L, L), :], out_hbm.at[pl.ds(s * L, L), :], 9 + s) for s in range(NSEG)]
    for c in (cx[0], cwk, cwq, cwv, cx[1], cwo, cx[2], cx[3]):
        c.start()

    gate = jax.nn.sigmoid(beta_ref[...].astype(F32))
    for j in range(H):
        GATE[j] = jnp.broadcast_to(gate[:, j:j + 1], (8, 128))
    wr8 = wr_ref[...].astype(F32)
    WR[...] = jnp.concatenate(
        [jnp.broadcast_to(wr8[c:c + 1, :], (16, 128)) for c in range(8)], axis=1).astype(BF)

    rowT = lax.broadcasted_iota(jnp.int32, (T, T), 0)
    colT = lax.broadcasted_iota(jnp.int32, (T, T), 1)

    never = GATE[0][0:1, 0:1] < -1.0
    def new_chain():
        return dict(never=never, tok=None) if CHAIN else None

    def ln1_pieces(s, chain=True):
        ch = new_chain() if chain else None
        def mk(r):
            def f():
                rows = slice(s * L + r * LNR, s * L + (r + 1) * LNR)
                XN[rows, :] = layernorm(X[rows, :].astype(F32), ch).astype(BF)
            return f
        return [mk(r) for r in range(L // LNR)]

    def ln2_pieces(s, chain_upto=99):
        ch = new_chain()
        def mk(r):
            def f():
                if r >= chain_upto:
                    ch["tok"] = None
                rows = slice(s * L + r * LNR, s * L + (r + 1) * LNR)
                xm = XM[rows, :].astype(F32)
                xn2 = layernorm(xm, ch).astype(BF)
                XN2[rows, :] = xn2
                xo = (xm + xn2.astype(F32)).astype(BF)
                X[rows, :] = xo
            return f
        return [mk(r) for r in range(L // LNR)]

    def r_pieces(s):
        def mk(c):
            def f():
                rows = slice(s * L + c * T, s * L + (c + 1) * T)
                rr = dot_nt(WR[...], XN2[rows, :])
                RALL[s * NT + c:s * NT + c + 1, :] = rr[0:1, :]
            return f
        return [mk(c) for c in range(NT)]

    def k_pieces(s):
        rows = slice(s * L, (s + 1) * L)
        def mk(g):
            def f():
                k = dot_nn(XN[rows, :], WK[:, g * T:(g + 1) * T])
                KK[g] = k.astype(BF)
                if s < NSEG - 1:
                    pk = phi(k)
                    PK[g] = pk.astype(BF)
                    z = jnp.sum(pk.reshape(L // 8, 8, 128), axis=0)
                    z = jnp.broadcast_to(jnp.sum(z, axis=0, keepdims=True), (8, 128))
                    ZZ[g] = z if s == 0 else ZZ[g] + z
            return f
        return [mk(g) for g in range(G)]

    def k_row_pieces(s):
        def mk(c):
            def f():
                rows = slice(s * L + c * T, s * L + (c + 1) * T)
                k = dot_nn(XN[rows, :], WK[...])
                for g in range(G):
                    kg = k[:, g * T:(g + 1) * T]
                    KK[g, c * T:(c + 1) * T, :] = kg.astype(BF)
                    if s < NSEG - 1:
                        pk = phi(kg)
                        PK[g, c * T:(c + 1) * T, :] = pk.astype(BF)
                        z = jnp.sum(pk.reshape(T // 8, 8, 128), axis=0)
                        ZZ[g] = z if (s == 0 and c == 0) else ZZ[g] + z
            return f
        return [mk(c) for c in range(NT)]

    def q_pieces(s):
        rows = slice(s * L, (s + 1) * L)
        def mk(g):
            def f():
                q = dot_nn(XN[rows, :], WQ[:, g * T:(g + 1) * T])
                QS[g] = (q * QSCALE).astype(BF)
                if s > 0:
                    PQ[g] = phi(q).astype(BF)
            return f
        return [mk(g) for g in range(G)]

    def v_pieces(s):
        def mk(hf, c):
            def f():
                vt = dot_nt(WVT[hf * L:(hf + 1) * L, :], XN[s * L + c * T:s * L + (c + 1) * T, :])
                for gg in range(4):
                    VT[hf * 4 + gg, :, c * T:(c + 1) * T] = vt[gg * T:(gg + 1) * T, :].astype(BF)
            return f
        return [mk(hf, c) for hf in range(2) for c in range(NT)]

    def o_pieces(s):
        rows = slice(s * L, (s + 1) * L)
        def mk(j):
            def f():
                o = jnp.concatenate([OB[g] for g in range(G)], axis=1)
                y = dot_nn(o, WO[:, j * T:(j + 1) * T])
                XM[rows, j * T:(j + 1) * T] = (X[rows, j * T:(j + 1) * T].astype(F32) + rb(y)).astype(BF)
            return f
        return [mk(j) for j in range(G)]

    def o_row_pieces(s):
        def mk(c):
            def f():
                rows = slice(s * L + c * T, s * L + (c + 1) * T)
                o = jnp.concatenate([OB[g, c * T:(c + 1) * T, :] for g in range(G)], axis=1)
                y = dot_nn(o, WO[...])
                XM[rows, :] = (X[rows, :].astype(F32) + rb(y)).astype(BF)
            return f
        return [mk(c) for c in range(NT)]

    def wvt_pieces():
        def mk(i):
            def f():
                for j in range(D // T):
                    WVT[j * T:(j + 1) * T, i * T:(i + 1) * T] = (
                        WV[i * T:(i + 1) * T, j * T:(j + 1) * T].astype(F32).T.astype(BF))
            return f
        return [mk(i) for i in range(D // T)]

    def mem_pieces(s):
        def retrieve(g):
            def f():
                r = dot_nt(AMEM[g], PQ[g])
                for h in range(4):
                    den = r[128 + 4 * h:129 + 4 * h, :] + 1e-6
                    OT[g, DH * h:DH * h + DH, :] = r[DH * h:DH * h + DH, :] * (GATE[4 * g + h][0:1, 0:1] / den)
            return f
        def update(g):
            def f():
                upd = dot_nn(VT[g], PK[g])
                rr = lax.broadcasted_iota(jnp.int32, (128, 128), 0) // DH
                cc = lax.broadcasted_iota(jnp.int32, (128, 128), 1) // DH
                upd = jnp.where(rr == cc, upd, 0.0)
                mt = upd if s == 0 else MT[g] + upd
                if s < NSEG - 2:
                    MT[g] = mt
                AMEM[g, 0:128, :] = mt.astype(BF)
                zr = lax.broadcasted_iota(jnp.int32, (16, 128), 0) // 4
                zc = lax.broadcasted_iota(jnp.int32, (16, 128), 1) // DH
                z = ZZ[g]
                AMEM[g, 128:144, :] = jnp.where(zr == zc, jnp.concatenate([z, z], axis=0), 0.0).astype(BF)
            return f
        out = []
        for g in range(G):
            if s > 0:
                out.append(retrieve(g))
            if s < NSEG - 1:
                out.append(update(g))
        return out

    def p1_steps(g, h, slot):
        state = {}
        def mk(qt, kt):
            def f():
                if kt == 0:
                    state["qm"] = head_mask(QS[g, qt * T:(qt + 1) * T, :], h)
                    state["m"] = None
                s = dot_nt(KK[g, kt * T:(kt + 1) * T, :], state["qm"])
                if kt == qt:
                    s = jnp.where(rowT <= colT, s, NEG)
                SB[slot, OFF[qt] + kt * T:OFF[qt] + (kt + 1) * T, :] = s
                mt = jnp.max(s.reshape(16, 8, 128), axis=0)
                state["m"] = mt if state["m"] is None else jnp.maximum(state["m"], mt)
                if kt == qt:
                    m = jnp.max(state["m"], axis=0, keepdims=True)
                    MB[slot, qt] = jnp.broadcast_to(m, (8, 128))
            return f
        return [mk(qt, kt) for qt in range(NT) for kt in range(qt + 1)]

    def p2_steps(g, h, slot, first_seg):
        state = {}
        def mk(qt, kt):
            def f():
                if kt == 0:
                    state["m"] = MB[slot, qt]
                    state["l"] = state["acc"] = None
                s = SB[slot, OFF[qt] + kt * T:OFF[qt] + (kt + 1) * T, :]
                p = jnp.exp2(s.reshape(16, 8, 128) - state["m"][None])
                ps = jnp.sum(p, axis=0)
                pv = dot_nn(VT[g, DH * h:DH * h + DH, kt * T:(kt + 1) * T],
                            p.reshape(T, 128).astype(BF))
                state["l"] = ps if state["l"] is None else state["l"] + ps
                state["acc"] = pv if state["acc"] is None else state["acc"] + pv
                if kt == qt:
                    lt = jnp.sum(state["l"], axis=0, keepdims=True)
                    w = (1.0 - GATE[4 * g + h][0:1, :]) / lt
                    res = state["acc"] * w
                    if not first_seg:
                        res = res + OT[g, DH * h:DH * h + DH, qt * T:(qt + 1) * T]
                    OT[g, DH * h:DH * h + DH, qt * T:(qt + 1) * T] = res
            return f
        return [mk(qt, kt) for qt in range(NT) for kt in range(qt + 1)]

    def tr_steps(g):
        def mk(qt):
            def f():
                OB[g, qt * T:(qt + 1) * T, :] = OT[g, :, qt * T:(qt + 1) * T].T.astype(BF)
            return f
        return [mk(qt) for qt in range(NT)]

    def attention(s):
        for g in range(G):
            for h in range(4):
                a = p2_steps(g, h, h % 2, s == 0)
                if h < 3:
                    b = p1_steps(g, h + 1, (h + 1) % 2)
                elif g < G - 1:
                    b = p1_steps(g + 1, 0, 0)
                else:
                    b = []
                t = tr_steps(g - 1) if (h == 0 and g > 0) else []
                for i in range(10):
                    a[i]()
                    if i < len(b):
                        b[i]()
                    if i < len(t):
                        t[i]()

    def routing_ffn(li):
        rv = rb(RALL[...])
        idx = (lax.broadcasted_iota(jnp.int32, (16, 128), 0) * 128
               + lax.broadcasted_iota(jnp.int32, (16, 128), 1))
        m1 = jnp.max(rv)
        i1 = jnp.clip(jnp.min(jnp.where(rv == m1, idx, S)), 0, S - 1)
        rv2 = jnp.where(idx == i1, -jnp.inf, rv)
        m2 = jnp.max(rv2)
        i2 = jnp.clip(jnp.min(jnp.where((rv2 == m2) & (idx != i1), idx, S)), 0, S - 1)
        row16 = lax.broadcasted_iota(jnp.int32, (16, D), 0)
        bases = [pl.multiple_of((i // 16) * 16, 16) for i in (i1, i2)]
        sel = []
        for i, base in zip((i1, i2), bases):
            blk = XN2[pl.ds(base, 16), :].astype(F32)
            sel.append(jnp.sum(jnp.where(row16 == i - base, blk, 0.0), axis=0, keepdims=True))
        xs = jnp.where(row16 == 0, sel[0], jnp.where(row16 == 1, sel[1], 0.0)).astype(BF)
        hs = []
        for j in range(NF):
            gg = rb(dot_nn(xs, WG[j]))
            uu = rb(dot_nn(xs, WU[j]))
            hs.append((rb(gg * jax.nn.sigmoid(gg)) * uu).astype(BF))
        hh = jnp.concatenate(hs, axis=1)
        ys = [dot_nn(hh, WD[n]) for n in range(D // T)]
        yy = rb(jnp.concatenate(ys, axis=1))
        for j, (i, base, mv) in enumerate(zip((i1, i2), bases, (m1, m2))):
            rs = rb(jax.nn.sigmoid(jnp.full((1, D), mv, F32)))
            upd = rb(yy[j:j + 1, :] * rs)
            blk = XN2[pl.ds(base, 16), :].astype(F32)
            nb = jnp.where(row16 == i - base, rb(blk + upd), blk)
            XN2[pl.ds(base, 16), :] = nb.astype(BF)
            xo = (XM[pl.ds(base, 16), :].astype(F32) + nb).astype(BF)
            X[pl.ds(base, 16), :] = xo
            if li == 0:
                XN[pl.ds(base, 16), :] = layernorm(xo.astype(F32)).astype(BF)
        return bases

    cx[0].wait()
    if not ONLY:
        for f in ln1_pieces(0, chain=False):
            f()
    cwk.wait()
    for li in range(2):
        first = li == 0
        for s in range(NSEG):
            if ONLY and ONLY != f"{li},{s}":
                continue
            kp, qp, vp = k_pieces(s), q_pieces(s), v_pieces(s)
            if s == 0:
                if first:
                    interleave(kp)
                    cwq.wait()
                    cwv.wait()
                    interleave(qp, wvt_pieces())
                    interleave(vp)
                else:
                    interleave(kp + qp + vp)
            else:
                for f in tr_steps(G - 1):
                    f()
                if first:
                    cx[s].wait()
                    if s == 1:
                        cwo.wait()
                        for c in cwg + cwu + cwd:
                            c.start()
                if VAR == "krow":
                    op, l1, kr = o_pieces(s - 1), ln1_pieces(s), k_row_pieces(s)
                    q4 = len(l1) // 4
                    for c in range(4):
                        interleave(op[2 * c:2 * c + 2], l1[c * q4:(c + 1) * q4])
                        kr[c]()
                    kp = []
                else:
                    interleave(o_pieces(s - 1), ln1_pieces(s))
                ln2, rp = ln2_pieces(s - 1), r_pieces(s - 1)
                q4 = len(ln2) // 4
                if kp:
                    interleave(kp[:4], ln2[0:q4])
                    interleave(kp[4:], ln2[q4:2 * q4])
                    rp[0]()
                    interleave(qp[:4], ln2[2 * q4:3 * q4])
                    rp[1]()
                    interleave(qp[4:], ln2[3 * q4:])
                    rp[2]()
                else:
                    interleave(qp[:3], ln2[0:q4])
                    rp[0]()
                    interleave(qp[3:6], ln2[q4:2 * q4])
                    rp[1]()
                    interleave(qp[6:] + vp[:1], ln2[2 * q4:3 * q4])
                    rp[2]()
                    interleave(vp[1:2], ln2[3 * q4:])
                    vp = vp[0:0] + vp[2:]
                interleave(vp[:2])
                rp[3]()
                if not first:
                    cout[s - 1].start()
                interleave(vp[2:])
            interleave(mem_pieces(s) + p1_steps(0, 0, 0))
            if ONLY:
                return
            lax.fori_loop(0, pl.program_id(0) + 1, lambda i, c, s=s: (attention(s), c)[1], 0)
        for f in tr_steps(G - 1):
            f()
        s = NSEG - 1
        op, ln2, rp = o_row_pieces(s), ln2_pieces(s, 12), r_pieces(s)
        op[0]()
        interleave([op[1]], ln2[0:4])
        interleave([op[2]], ln2[4:8])
        rp[0]()
        interleave([op[3]], ln2[8:12])
        rp[1]()
        rp[2]()
        interleave(ln2[12:16])
        rp[3]()
        if not first:
            cout[s].start()
        if first:
            for c in cwg + cwu + cwd:
                c.wait()
            interleave(ln1_pieces(0))
        bases = routing_ffn(li)
        if not first:
            for c in cout:
                c.wait()
            p0 = pltpu.make_async_copy(X.at[pl.ds(bases[0], 16), :], out_hbm.at[pl.ds(bases[0], 16), :], sems.at[13])
            p1 = pltpu.make_async_copy(X.at[pl.ds(bases[1], 16), :], out_hbm.at[pl.ds(bases[1], 16), :], sems.at[14])
            p0.start()
            @pl.when(bases[1] != bases[0])
            def _():
                p1.start()
                p1.wait()
            p0.wait()


@jax.jit
def pallas_interleave_layers__memory_aug_infini_attn__moe_arch_mod__prompt_kernel(
    A_x, A_wq, A_wk, A_wv, A_wo, A_beta, B_x, B_w_r, B_w_gate, B_w_up, B_w_down):
    del B_x
    any_spec = pl.BlockSpec(memory_space=pl.ANY)
    vm = pltpu.VMEM
    blk = vm((G, L, 128), BF)
    out = pl.pallas_call(
        kernel,
        out_shape=jax.ShapeDtypeStruct((S, D), BF),
        grid=(1,),
        in_specs=[any_spec, any_spec, any_spec, any_spec, any_spec,
                  pl.BlockSpec((1, H), lambda i: (0, 0)), pl.BlockSpec((8, 128), lambda i: (0, 0)),
                  any_spec, any_spec, any_spec],
        out_specs=any_spec,
        scratch_shapes=[
            vm((S, D), BF), vm((S, D), BF), vm((S, D), BF), vm((S, D), BF),
            vm((D, D), BF), vm((D, D), BF), vm((D, D), BF), vm((D, D), BF), vm((D, D), BF),
            vm((NF, D, T), BF), vm((NF, D, T), BF), vm((D // T, F, T), BF),
            blk, blk, blk, blk, vm((G, 128, L), BF),
            vm((2, 1280, 128), F32), vm((2, NT, 8, 128), F32),
            vm((G, 128, L), F32), blk,
            vm((G, 128, 128), F32), vm((G, 8, 128), F32), vm((G, 144, 128), BF),
            vm((H, 8, 128), F32), vm((16, D), BF), vm((16, 128), F32),
            pltpu.SemaphoreType.DMA((15,)),
        ],
        compiler_params=pltpu.CompilerParams(vmem_limit_bytes=110 * 1024 * 1024, flags=FLAGS),
        name="fused",
    )(A_x.reshape(S, D), A_wq, A_wk, A_wv, A_wo, A_beta.reshape(1, H), B_w_r.reshape(8, 128),
      B_w_gate, B_w_up, B_w_down)
    return out.reshape(1, S, D)
```

```python
import jax
import jax.numpy as jnp
import numpy as np
from jax import lax
import jax.experimental.pallas as pl
import jax.experimental.pallas.tpu as pltpu

S, D, F = 2048, 1024, 3584
H, DH = 32, 32
NSEG, L = 4, 512
G, T = 8, 128
NT = L // T
NF = F // T
OFF = (0, 128, 384, 768)
NEG = -1e30
EPS = 1e-5
QSCALE = float(DH ** -0.5 * np.log2(np.e))
BF = jnp.bfloat16
F32 = jnp.float32
import os
LNR = int(os.environ.get('LNR', '32'))
ONLY = os.environ.get('ONLY')
VAR = os.environ.get('VAR', '')
CHAIN = int(os.environ.get('CHAIN', '1'))
FLAGS = {k: True for k in os.environ.get('FLAGS', '').split(',') if k} or None


def dot_nt(a, b):
    return lax.dot_general(a, b, (((1,), (1,)), ((), ())), preferred_element_type=F32)


def dot_nn(a, b):
    return lax.dot_general(a, b, (((1,), (0,)), ((), ())), preferred_element_type=F32)


def rb(x):
    return x.astype(BF).astype(F32)


def layernorm(x, chain=None):
    m = jnp.sum(x, axis=-1, keepdims=True) * (1.0 / D)
    if chain is not None and chain.get("tok") is not None:
        m = jnp.where(chain["never"], chain["tok"], m)
    c = x - m
    v = jnp.sum(c * c, axis=-1, keepdims=True) * (1.0 / D)
    a = rb(rb(v) + EPS)
    y = lax.rsqrt(a)
    s = rb(a * y)
    y = y * (2.0 - s * y)
    if chain is not None:
        chain["tok"] = y
    return c * y


def phi(t):
    return jnp.where(t > 0, t + 1.0, jnp.exp(t))


def head_mask(x, h):
    u = pltpu.bitcast(x, jnp.uint32)
    lane = lax.broadcasted_iota(jnp.int32, u.shape, 1)
    u = jnp.where((lane >= DH * h) & (lane < DH * h + DH), u, jnp.uint32(0))
    return pltpu.bitcast(u, BF)


def interleave(main, *bgs):
    main = list(main)
    bgs = [list(b) for b in bgs]
    done = [0] * len(bgs)
    n = len(main)
    for i, piece in enumerate(main):
        piece()
        for bi, b in enumerate(bgs):
            upto = (i + 1) * len(b) // n
            while done[bi] < upto:
                b[done[bi]]()
                done[bi] += 1


def kernel(x_hbm, wq_hbm, wk_hbm, wv_hbm, wo_hbm, beta_ref, wr_ref, wg_hbm, wu_hbm, wd_hbm,
           out_hbm,
           X, XM, XN2, XN, WQ, WK, WV, WVT, WO, WG, WU, WD,
           QS, KK, PQ, PK, VT, SB, MB, OT, OB, MT, ZZ, AMEM, GATE, WR, RALL, sems):
    def cp(src, dst, i):
        return pltpu.make_async_copy(src, dst, sems.at[i])
    cx = [cp(x_hbm.at[pl.ds(s * L, L), :], X.at[pl.ds(s * L, L), :], s) for s in range(NSEG)]
    cwq, cwk, cwv, cwo = (cp(wq_hbm, WQ, 4), cp(wk_hbm, WK, 5), cp(wv_hbm, WV, 6), cp(wo_hbm, WO, 7))
    cwg = [cp(wg_hbm.at[:, pl.ds(j * T, T)], WG.at[j], 8) for j in range(NF)]
    cwu = [cp(wu_hbm.at[:, pl.ds(j * T, T)], WU.at[j], 8) for j in range(NF)]
    cwd = [cp(wd_hbm.at[:, pl.ds(j * T, T)], WD.at[j], 8) for j in range(D // T)]
    cout = [cp(X.at[pl.ds(s * L, L), :], out_hbm.at[pl.ds(s * L, L), :], 9 + s) for s in range(NSEG)]
    SV = os.environ.get("SV", "2")
    cx0 = [cp(x_hbm.at[pl.ds(c * T, T), :], X.at[pl.ds(c * T, T), :], 15 + c) for c in range(NT)]
    cwkc = [cp(wk_hbm.at[:, pl.ds(g * T, T)], WK.at[:, pl.ds(g * T, T)], 19 + g) for g in range(G)]
    if SV == "0":
        cx[0].start()
        cwk.start()
    elif SV == "1":
        cx[0].start()
        for c in cwkc: c.start()
    elif SV == "2":
        for c in cx0: c.start()
        for c in cwkc: c.start()
    elif SV == "3":
        for c in cx0: c.start()
    elif SV == "4":
        cx[0].start()

    gate = jax.nn.sigmoid(beta_ref[...].astype(F32))
    for j in range(H):
        GATE[j] = jnp.broadcast_to(gate[:, j:j + 1], (8, 128))
    wr8 = wr_ref[...].astype(F32)
    WR[...] = jnp.concatenate(
        [jnp.broadcast_to(wr8[c:c + 1, :], (16, 128)) for c in range(8)], axis=1).astype(BF)

    rowT = lax.broadcasted_iota(jnp.int32, (T, T), 0)
    colT = lax.broadcasted_iota(jnp.int32, (T, T), 1)

    never = GATE[0][0:1, 0:1] < -1.0
    def new_chain():
        return dict(never=never, tok=None) if CHAIN else None

    def ln1_pieces(s, chain=True):
        ch = new_chain() if chain else None
        def mk(r):
            def f():
                rows = slice(s * L + r * LNR, s * L + (r + 1) * LNR)
                XN[rows, :] = layernorm(X[rows, :].astype(F32), ch).astype(BF)
            return f
        return [mk(r) for r in range(L // LNR)]

    def ln2_pieces(s, chain_upto=99):
        ch = new_chain()
        def mk(r):
            def f():
                if r >= chain_upto:
                    ch["tok"] = None
                rows = slice(s * L + r * LNR, s * L + (r + 1) * LNR)
                xm = XM[rows, :].astype(F32)
                xn2 = layernorm(xm, ch).astype(BF)
                XN2[rows, :] = xn2
                xo = (xm + xn2.astype(F32)).astype(BF)
                X[rows, :] = xo
            return f
        return [mk(r) for r in range(L // LNR)]

    def r_pieces(s):
        def mk(c):
            def f():
                rows = slice(s * L + c * T, s * L + (c + 1) * T)
                rr = dot_nt(WR[...], XN2[rows, :])
                RALL[s * NT + c:s * NT + c + 1, :] = rr[0:1, :]
            return f
        return [mk(c) for c in range(NT)]

    def k_pieces(s):
        rows = slice(s * L, (s + 1) * L)
        def mk(g):
            def f():
                k = dot_nn(XN[rows, :], WK[:, g * T:(g + 1) * T])
                KK[g] = k.astype(BF)
                if s < NSEG - 1:
                    pk = phi(k)
                    PK[g] = pk.astype(BF)
                    z = jnp.sum(pk.reshape(L // 8, 8, 128), axis=0)
                    z = jnp.broadcast_to(jnp.sum(z, axis=0, keepdims=True), (8, 128))
                    ZZ[g] = z if s == 0 else ZZ[g] + z
            return f
        return [mk(g) for g in range(G)]

    def k_row_pieces(s):
        def mk(c):
            def f():
                rows = slice(s * L + c * T, s * L + (c + 1) * T)
                k = dot_nn(XN[rows, :], WK[...])
                for g in range(G):
                    kg = k[:, g * T:(g + 1) * T]
                    KK[g, c * T:(c + 1) * T, :] = kg.astype(BF)
                    if s < NSEG - 1:
                        pk = phi(kg)
                        PK[g, c * T:(c + 1) * T, :] = pk.astype(BF)
                        z = jnp.sum(pk.reshape(T // 8, 8, 128), axis=0)
                        ZZ[g] = z if (s == 0 and c == 0) else ZZ[g] + z
            return f
        return [mk(c) for c in range(NT)]

    def q_pieces(s):
        rows = slice(s * L, (s + 1) * L)
        def mk(g):
            def f():
                q = dot_nn(XN[rows, :], WQ[:, g * T:(g + 1) * T])
                QS[g] = (q * QSCALE).astype(BF)
                if s > 0:
                    PQ[g] = phi(q).astype(BF)
            return f
        return [mk(g) for g in range(G)]

    def v_pieces(s):
        def mk(hf, c):
            def f():
                vt = dot_nt(WVT[hf * L:(hf + 1) * L, :], XN[s * L + c * T:s * L + (c + 1) * T, :])
                for gg in range(4):
                    VT[hf * 4 + gg, :, c * T:(c + 1) * T] = vt[gg * T:(gg + 1) * T, :].astype(BF)
            return f
        return [mk(hf, c) for hf in range(2) for c in range(NT)]

    def o_pieces(s):
        rows = slice(s * L, (s + 1) * L)
        def mk(j):
            def f():
                o = jnp.concatenate([OB[g] for g in range(G)], axis=1)
                y = dot_nn(o, WO[:, j * T:(j + 1) * T])
                XM[rows, j * T:(j + 1) * T] = (X[rows, j * T:(j + 1) * T].astype(F32) + rb(y)).astype(BF)
            return f
        return [mk(j) for j in range(G)]

    def o_row_pieces(s):
        def mk(c):
            def f():
                rows = slice(s * L + c * T, s * L + (c + 1) * T)
                o = jnp.concatenate([OB[g, c * T:(c + 1) * T, :] for g in range(G)], axis=1)
                y = dot_nn(o, WO[...])
                XM[rows, :] = (X[rows, :].astype(F32) + rb(y)).astype(BF)
            return f
        return [mk(c) for c in range(NT)]

    def wvt_pieces():
        def mk(i):
            def f():
                for j in range(D // T):
                    WVT[j * T:(j + 1) * T, i * T:(i + 1) * T] = (
                        WV[i * T:(i + 1) * T, j * T:(j + 1) * T].astype(F32).T.astype(BF))
            return f
        return [mk(i) for i in range(D // T)]

    def mem_pieces(s):
        def retrieve(g):
            def f():
                r = dot_nt(AMEM[g], PQ[g])
                for h in range(4):
                    den = r[128 + 4 * h:129 + 4 * h, :] + 1e-6
                    OT[g, DH * h:DH * h + DH, :] = r[DH * h:DH * h + DH, :] * (GATE[4 * g + h][0:1, 0:1] / den)
            return f
        def update(g):
            def f():
                upd = dot_nn(VT[g], PK[g])
                rr = lax.broadcasted_iota(jnp.int32, (128, 128), 0) // DH
                cc = lax.broadcasted_iota(jnp.int32, (128, 128), 1) // DH
                upd = jnp.where(rr == cc, upd, 0.0)
                mt = upd if s == 0 else MT[g] + upd
                if s < NSEG - 2:
                    MT[g] = mt
                AMEM[g, 0:128, :] = mt.astype(BF)
                zr = lax.broadcasted_iota(jnp.int32, (16, 128), 0) // 4
                zc = lax.broadcasted_iota(jnp.int32, (16, 128), 1) // DH
                z = ZZ[g]
                AMEM[g, 128:144, :] = jnp.where(zr == zc, jnp.concatenate([z, z], axis=0), 0.0).astype(BF)
            return f
        ret = [retrieve(g) for g in range(G)] if s > 0 else []
        upd = [update(g) for g in range(G)] if s < NSEG - 1 else []
        return ret, upd

    def p1_steps(g, h, slot, qord='0123'):
        state = {}
        def mk(qt, kt):
            def f():
                if kt == 0:
                    state["qm"] = head_mask(QS[g, qt * T:(qt + 1) * T, :], h)
                    state["m"] = None
                s = dot_nt(KK[g, kt * T:(kt + 1) * T, :], state["qm"])
                if kt == qt:
                    s = jnp.where(rowT <= colT, s, NEG)
                SB[slot, OFF[qt] + kt * T:OFF[qt] + (kt + 1) * T, :] = s
                mt = jnp.max(s.reshape(16, 8, 128), axis=0)
                state["m"] = mt if state["m"] is None else jnp.maximum(state["m"], mt)
                if kt == qt:
                    m = jnp.max(state["m"], axis=0, keepdims=True)
                    MB[slot, qt] = jnp.broadcast_to(m, (8, 128))
            return f
        return [mk(int(qt), kt) for qt in qord for kt in range(int(qt) + 1)]

    def p2_steps(g, h, slot, first_seg, qord='0123'):
        state = {}
        def mk(qt, kt):
            def f():
                if kt == 0:
                    state["m"] = MB[slot, qt]
                    state["l"] = state["acc"] = None
                s = SB[slot, OFF[qt] + kt * T:OFF[qt] + (kt + 1) * T, :]
                p = jnp.exp2(s.reshape(16, 8, 128) - state["m"][None])
                ps = jnp.sum(p, axis=0)
                pv = dot_nn(VT[g, DH * h:DH * h + DH, kt * T:(kt + 1) * T],
                            p.reshape(T, 128).astype(BF))
                state["l"] = ps if state["l"] is None else state["l"] + ps
                state["acc"] = pv if state["acc"] is None else state["acc"] + pv
                if kt == qt:
                    lt = jnp.sum(state["l"], axis=0, keepdims=True)
                    w = (1.0 - GATE[4 * g + h][0:1, :]) / lt
                    res = state["acc"] * w
                    if not first_seg:
                        res = res + OT[g, DH * h:DH * h + DH, qt * T:(qt + 1) * T]
                    OT[g, DH * h:DH * h + DH, qt * T:(qt + 1) * T] = res
            return f
        return [mk(int(qt), kt) for qt in qord for kt in range(int(qt) + 1)]

    def tr_steps(g):
        def mk(qt):
            def f():
                OB[g, qt * T:(qt + 1) * T, :] = OT[g, :, qt * T:(qt + 1) * T].T.astype(BF)
            return f
        return [mk(qt) for qt in range(NT)]

    def attention(s):
        AV = os.environ.get("AV", "12")
        Q1, Q2 = os.environ.get("Q1", "1302"), os.environ.get("Q2", "1302")
        seq_a, seq_b = [], []
        for g in range(G):
            for h in range(4):
                a = p2_steps(g, h, h % 2, s == 0, Q2)
                if h < 3:
                    b = p1_steps(g, h + 1, (h + 1) % 2, Q1)
                elif g < G - 1:
                    b = p1_steps(g + 1, 0, 0, Q1)
                else:
                    b = mem_pieces(s)[1]
                t = tr_steps(g - 1) if (h == 0 and g > 0) else []
                if AV == "21":
                    for i in range(10):
                        a[i]()
                        if i < len(b): b[i]()
                        if i < len(t): t[i]()
                elif AV == "12":
                    for i in range(10):
                        if i < len(b): b[i]()
                        a[i]()
                        if i < len(t): t[i]()
                elif AV == "2211":
                    for i in range(0, 10, 2):
                        a[i](); a[i + 1]()
                        if i < len(b): b[i](); b[i + 1]()
                        if i // 2 < len(t): t[i // 2]()
                elif AV == "ser21":
                    for f in a: f()
                    for f in b: f()
                    for f in t: f()
                elif AV == "ser12":
                    for f in b: f()
                    for f in a: f()
                    for f in t: f()

    def routing_ffn(li):
        rv = rb(RALL[...])
        idx = (lax.broadcasted_iota(jnp.int32, (16, 128), 0) * 128
               + lax.broadcasted_iota(jnp.int32, (16, 128), 1))
        m1 = jnp.max(rv)
        i1 = jnp.clip(jnp.min(jnp.where(rv == m1, idx, S)), 0, S - 1)
        rv2 = jnp.where(idx == i1, -jnp.inf, rv)
        m2 = jnp.max(rv2)
        i2 = jnp.clip(jnp.min(jnp.where((rv2 == m2) & (idx != i1), idx, S)), 0, S - 1)
        row16 = lax.broadcasted_iota(jnp.int32, (16, D), 0)
        bases = [pl.multiple_of((i // 16) * 16, 16) for i in (i1, i2)]
        sel = []
        for i, base in zip((i1, i2), bases):
            blk = XN2[pl.ds(base, 16), :].astype(F32)
            sel.append(jnp.sum(jnp.where(row16 == i - base, blk, 0.0), axis=0, keepdims=True))
        xs = jnp.where(row16 == 0, sel[0], jnp.where(row16 == 1, sel[1], 0.0)).astype(BF)
        hs = []
        for j in range(NF):
            gg = rb(dot_nn(xs, WG[j]))
            uu = rb(dot_nn(xs, WU[j]))
            hs.append((rb(gg * jax.nn.sigmoid(gg)) * uu).astype(BF))
        hh = jnp.concatenate(hs, axis=1)
        ys = [dot_nn(hh, WD[n]) for n in range(D // T)]
        yy = rb(jnp.concatenate(ys, axis=1))
        for j, (i, base, mv) in enumerate(zip((i1, i2), bases, (m1, m2))):
            rs = rb(jax.nn.sigmoid(jnp.full((1, D), mv, F32)))
            upd = rb(yy[j:j + 1, :] * rs)
            blk = XN2[pl.ds(base, 16), :].astype(F32)
            nb = jnp.where(row16 == i - base, rb(blk + upd), blk)
            XN2[pl.ds(base, 16), :] = nb.astype(BF)
            xo = (XM[pl.ds(base, 16), :].astype(F32) + nb).astype(BF)
            X[pl.ds(base, 16), :] = xo
            if li == 0:
                XN[pl.ds(base, 16), :] = layernorm(xo.astype(F32)).astype(BF)
        return bases

    def block_b(li, s):
        first = li == 0
        kp, qp, vp = k_pieces(s), q_pieces(s), v_pieces(s)
        ret = mem_pieces(s)[0]
        p10 = p1_steps(0, 0, 0, os.environ.get("QB", "0123"))
        if s == 0:
            if first:
                if SV in ("0",) or (ONLY and ONLY != "START"):
                    interleave(kp)
                else:
                    for g in range(G):
                        cwkc[g].wait()
                        if g == 1:
                            cwv.start()
                        kp[g]()
                cwq.wait()
                for c in (cx[1], cwo, cx[2], cx[3]):
                    c.start()
                interleave(qp[:4])
                cwv.wait()
                interleave(qp[4:], wvt_pieces())
                interleave(vp, p10)
            else:
                interleave(kp + qp)
                interleave(vp, p10)
        else:
            for f in tr_steps(G - 1):
                f()
            if first and not ONLY:
                cx[s].wait()
                if s == 1:
                    cwo.wait()
                    for c in cwg + cwu + cwd:
                        c.start()
            interleave(o_pieces(s - 1), ln1_pieces(s))
            ln2, rp = ln2_pieces(s - 1), r_pieces(s - 1)
            q4 = len(ln2) // 4
            interleave(kp[:4], ln2[0:q4])
            interleave(kp[4:], ln2[q4:2 * q4])
            rp[0]()
            interleave(qp[:4], ln2[2 * q4:3 * q4])
            rp[1]()
            interleave(qp[4:], ln2[3 * q4:])
            rp[2]()
            interleave(vp[:2])
            rp[3]()
            if not first and not ONLY:
                cout[s - 1].start()
            BV = os.environ.get("BV", "3")
            if BV == "0":
                interleave(vp[2:], ret + p10)
            elif BV == "1":
                interleave(vp[2:], p10 + ret)
            elif BV == "2":
                interleave(vp[2:], p10, ret)
            elif BV == "3":
                interleave(vp[2:6], ret)
                interleave(vp[6:], p10)
            elif BV == "4":
                interleave(vp[2:])
                interleave(ret + p10)

    def block_t(li):
        first = li == 0
        for f in tr_steps(G - 1):
            f()
        s = NSEG - 1
        TV = os.environ.get("TV", "0")
        op, ln2, rp = o_row_pieces(s), ln2_pieces(s, int(os.environ.get("TC", "12"))), r_pieces(s)
        if TV == "0":
            op[0]()
            interleave([op[1]], ln2[0:4])
            interleave([op[2]], ln2[4:8])
            rp[0]()
            interleave([op[3]], ln2[8:12])
            rp[1]()
            rp[2]()
            interleave(ln2[12:16])
            rp[3]()
        elif TV == "1":
            op[0]()
            interleave([op[1]], ln2[0:4])
            rp[0]()
            interleave([op[2]], ln2[4:8])
            rp[1]()
            interleave([op[3]], ln2[8:12])
            rp[2]()
            interleave(ln2[12:16])
            rp[3]()
        if not first and not ONLY:
            cout[s].start()

    def block_f(li):
        routing_ffn(li)

    def block_a(li, s):
        attention(s)

    def cut(fn):
        lax.fori_loop(0, pl.program_id(0) + 1, lambda i, c: (fn(), c)[1], 0)

    def startup():
        l1 = ln1_pieces(0, chain=False)
        if SV == "0":
            cx[0].wait()
            cwq.start()
            for f in l1: f()
            cwk.wait()
            cwv.start()
        elif SV == "1":
            cx[0].wait()
            cwq.start()
            for f in l1: f()
        elif SV == "2":
            n = len(l1) // NT
            for c in range(NT):
                cx0[c].wait()
                if c == NT - 1:
                    cwq.start()
                for f in l1[c * n:(c + 1) * n]: f()
        elif SV == "3":
            n = len(l1) // NT
            for c in range(NT):
                cx0[c].wait()
                if c == 0:
                    for cc in cwkc: cc.start()
                if c == NT - 1:
                    cwq.start()
                for f in l1[c * n:(c + 1) * n]: f()
        elif SV == "4":
            cx[0].wait()
            for cc in cwkc: cc.start()
            cwq.start()
            for f in l1: f()

    if ONLY == "START":
        startup()
        block_b(0, 0)
        for c in (cx[1], cwo, cx[2], cx[3]):
            c.wait()
        return
    if ONLY:
        for item in ONLY.split(";"):
            def run(item=item):
                for name in item.strip("[").split("+"):
                    if name[0] == "T":
                        block_t(int(name[1]))
                        continue
                    if name[0] == "F":
                        block_f(int(name[1]))
                        continue
                    li, s = int(name[1]), int(name[2])
                    (block_a if name[0] == "A" else block_b)(li, s)
            if item.startswith("["):
                cut(run)
            else:
                run()
        cx[0].wait()
        cwk.wait()
        return

    startup()
    for li in range(2):
        first = li == 0
        for s in range(NSEG):
            block_b(li, s)
            cut(lambda: block_a(li, s))
        block_t(li)
        if first:
            for c in cwg + cwu + cwd:
                c.wait()
            interleave(ln1_pieces(0))
        bases = routing_ffn(li)
        if not first:
            for c in cout:
                c.wait()
            p0 = pltpu.make_async_copy(X.at[pl.ds(bases[0], 16), :], out_hbm.at[pl.ds(bases[0], 16), :], sems.at[13])
            p1 = pltpu.make_async_copy(X.at[pl.ds(bases[1], 16), :], out_hbm.at[pl.ds(bases[1], 16), :], sems.at[14])
            p0.start()
            @pl.when(bases[1] != bases[0])
            def _():
                p1.start()
                p1.wait()
            p0.wait()


@jax.jit
def pallas_interleave_layers__memory_aug_infini_attn__moe_arch_mod__prompt_kernel(
    A_x, A_wq, A_wk, A_wv, A_wo, A_beta, B_x, B_w_r, B_w_gate, B_w_up, B_w_down):
    del B_x
    any_spec = pl.BlockSpec(memory_space=pl.ANY)
    vm = pltpu.VMEM
    blk = vm((G, L, 128), BF)
    out = pl.pallas_call(
        kernel,
        out_shape=jax.ShapeDtypeStruct((S, D), BF),
        grid=(1,),
        in_specs=[any_spec, any_spec, any_spec, any_spec, any_spec,
                  pl.BlockSpec((1, H), lambda i: (0, 0)), pl.BlockSpec((8, 128), lambda i: (0, 0)),
                  any_spec, any_spec, any_spec],
        out_specs=any_spec,
        scratch_shapes=[
            vm((S, D), BF), vm((S, D), BF), vm((S, D), BF), vm((S, D), BF),
            vm((D, D), BF), vm((D, D), BF), vm((D, D), BF), vm((D, D), BF), vm((D, D), BF),
            vm((NF, D, T), BF), vm((NF, D, T), BF), vm((D // T, F, T), BF),
            blk, blk, blk, blk, vm((G, 128, L), BF),
            vm((2, 1280, 128), F32), vm((2, NT, 8, 128), F32),
            vm((G, 128, L), F32), blk,
            vm((G, 128, 128), F32), vm((G, 8, 128), F32), vm((G, 144, 128), BF),
            vm((H, 8, 128), F32), vm((16, D), BF), vm((16, 128), F32),
            pltpu.SemaphoreType.DMA((27,)),
        ],
        compiler_params=pltpu.CompilerParams(vmem_limit_bytes=110 * 1024 * 1024, flags=FLAGS),
        name="fused",
    )(A_x.reshape(S, D), A_wq, A_wk, A_wv, A_wo, A_beta.reshape(1, H), B_w_r.reshape(8, 128),
      B_w_gate, B_w_up, B_w_down)
    return out.reshape(1, S, D)
```

```python
import jax
import jax.numpy as jnp
import numpy as np
from jax import lax
import jax.experimental.pallas as pl
import jax.experimental.pallas.tpu as pltpu

S, D, F = 2048, 1024, 3584
H, DH = 32, 32
NSEG, L = 4, 512
G, T = 8, 128
NT = L // T
NF = F // T
OFF = (0, 128, 384, 768)
NEG = -1e30
EPS = 1e-5
QSCALE = float(DH ** -0.5 * np.log2(np.e))
BF = jnp.bfloat16
F32 = jnp.float32
import os
LNR = int(os.environ.get('LNR', '32'))
ONLY = os.environ.get('ONLY')
VAR = os.environ.get('VAR', '')
CHAIN = int(os.environ.get('CHAIN', '1'))
FLAGS = {k: True for k in os.environ.get('FLAGS', '').split(',') if k} or None


def dot_nt(a, b):
    return lax.dot_general(a, b, (((1,), (1,)), ((), ())), preferred_element_type=F32)


def dot_nn(a, b):
    return lax.dot_general(a, b, (((1,), (0,)), ((), ())), preferred_element_type=F32)


def rb(x):
    return x.astype(BF).astype(F32)


def layernorm(x, chain=None):
    m = jnp.sum(x, axis=-1, keepdims=True) * (1.0 / D)
    if chain is not None and chain.get("tok") is not None:
        m = jnp.where(chain["never"], chain["tok"], m)
    c = x - m
    v = jnp.sum(c * c, axis=-1, keepdims=True) * (1.0 / D)
    a = rb(rb(v) + EPS)
    y = lax.rsqrt(a)
    s = rb(a * y)
    y = y * (2.0 - s * y)
    if chain is not None:
        chain["tok"] = y
    return c * y


def gate_rows(x, chain):
    if chain is None or chain.get("tok") is None:
        return x
    u = pltpu.bitcast(x, jnp.uint32)
    t = pltpu.bitcast(chain["tok"], jnp.uint32)
    t = jnp.concatenate([t] * (u.shape[1] // 128), axis=1)
    t = jnp.concatenate([t] * (u.shape[0] // 8), axis=0)
    return pltpu.bitcast(jnp.where(chain["never"], t, u), BF)


def phi(t):
    return jnp.where(t > 0, t + 1.0, jnp.exp(t))


def head_mask(x, h):
    u = pltpu.bitcast(x, jnp.uint32)
    lane = lax.broadcasted_iota(jnp.int32, u.shape, 1)
    u = jnp.where((lane >= DH * h) & (lane < DH * h + DH), u, jnp.uint32(0))
    return pltpu.bitcast(u, BF)


def interleave(main, *bgs):
    main = list(main)
    bgs = [list(b) for b in bgs]
    done = [0] * len(bgs)
    n = len(main)
    for i, piece in enumerate(main):
        piece()
        for bi, b in enumerate(bgs):
            upto = (i + 1) * len(b) // n
            while done[bi] < upto:
                b[done[bi]]()
                done[bi] += 1


def kernel(x_hbm, wq_hbm, wk_hbm, wv_hbm, wo_hbm, beta_ref, wr_ref, wg_hbm, wu_hbm, wd_hbm,
           out_hbm,
           X, XM, XN2, XN, WQ, WK, WV, WVT, WO, WG, WU, WD,
           QS, KK, PQ, PK, VT, SB, MB, OT, OB, MT, ZZ, AMEM, GATE, WR, WRB, TOP, RALL, sems):
    def cp(src, dst, i):
        return pltpu.make_async_copy(src, dst, sems.at[i])
    cx = [cp(x_hbm.at[pl.ds(s * L, L), :], X.at[pl.ds(s * L, L), :], s) for s in range(NSEG)]
    cwq, cwk, cwv, cwo = (cp(wq_hbm, WQ, 4), cp(wk_hbm, WK, 5), cp(wv_hbm, WV, 6), cp(wo_hbm, WO, 7))
    cwd = [cp(wd_hbm.at[:, pl.ds(j * T, T)], WD.at[j], 28) for j in range(D // T)]
    cwg = [cp(wg_hbm, WG, 8)]
    cwu = [cp(wu_hbm, WU, 27)]
    cout = [cp(X.at[pl.ds(s * L, L), :], out_hbm.at[pl.ds(s * L, L), :], 9 + s) for s in range(NSEG)]
    SV = os.environ.get("SV", "2")
    cx0 = [cp(x_hbm.at[pl.ds(c * T, T), :], X.at[pl.ds(c * T, T), :], 15 + c) for c in range(NT)]
    cwkc = [cp(wk_hbm.at[:, pl.ds(g * T, T)], WK.at[:, pl.ds(g * T, T)], 19 + g) for g in range(G)]
    if SV == "0":
        cx[0].start()
        cwk.start()
    elif SV == "1":
        cx[0].start()
        for c in cwkc: c.start()
    elif SV == "2":
        for c in cx0: c.start()
        for c in cwkc: c.start()
    elif SV == "3":
        for c in cx0: c.start()
    elif SV == "4":
        cx[0].start()

    gate = jax.nn.sigmoid(beta_ref[...].astype(F32))
    for j in range(H):
        GATE[j] = jnp.broadcast_to(gate[:, j:j + 1], (8, 128))
    wr8 = wr_ref[...].astype(F32)
    WR[...] = jnp.concatenate(
        [jnp.broadcast_to(wr8[c:c + 1, :], (8, 128)) for c in range(8)], axis=1)
    WRB[...] = jnp.concatenate(
        [jnp.broadcast_to(wr8[c:c + 1, :], (16, 128)) for c in range(8)], axis=1).astype(BF)
    RALL[...] = jnp.full(RALL.shape, jnp.iinfo(jnp.int32).min, jnp.int32)

    rowT = lax.broadcasted_iota(jnp.int32, (T, T), 0)
    colT = lax.broadcasted_iota(jnp.int32, (T, T), 1)

    never = GATE[0][0:1, 0:1] < -1.0
    PACE = False
    pace = dict(ch=None)
    def set_pace(val):
        if PACE and pace["ch"] is not None:
            pace["ch"]["tok"] = val[0:8, 0:128]
    def new_chain():
        return dict(never=never, tok=None) if CHAIN else None

    def ln1_pieces(s, chain=True):
        ch = new_chain() if chain else None
        pace["ch"] = ch
        def mk(r):
            def f():
                rows = slice(s * L + r * LNR, s * L + (r + 1) * LNR)
                XN[rows, :] = layernorm(X[rows, :].astype(F32), ch).astype(BF)
            return f
        return [mk(r) for r in range(L // LNR)]

    def score_key(sc, tok):
        u = pltpu.bitcast(sc, jnp.int32)
        return (u ^ ((u >> 31) & 0x7FFF0000)) | (0xFFFF - tok)

    def ln2_pieces(s, chain_upto=99, route=False):
        ch = new_chain()
        nrg = LNR // 8
        def mk(r):
            def f():
                if r >= chain_upto:
                    ch["tok"] = None
                r0 = s * L + r * LNR
                rows = slice(r0, r0 + LNR)
                xm = XM[rows, :].astype(F32)
                xn2 = layernorm(xm, ch).astype(BF)
                XN2[rows, :] = xn2
                xf = xn2.astype(F32)
                X[rows, :] = (xm + xf).astype(BF)
                if route:
                    prod = xf.reshape(nrg, 8, D) * WR[...][None]
                    sc = rb(jnp.sum(prod, axis=-1, keepdims=True))
                    sc = jnp.broadcast_to(sc, (nrg, 8, 128)).reshape(LNR, 128)
                    key = score_key(sc, r0 + lax.broadcasted_iota(jnp.int32, (LNR, 128), 0))
                    t1, t2 = TOP[0], TOP[1]
                    for j in range(nrg):
                        kj = key[8 * j:8 * j + 8]
                        t2 = jnp.maximum(t2, jnp.minimum(t1, kj))
                        t1 = jnp.maximum(t1, kj)
                    TOP[0] = t1
                    TOP[1] = t2
            return f
        return [mk(r) for r in range(L // LNR)]

    def r_pieces(s):
        def mk(c):
            def f():
                r0 = s * L + c * T
                rr = dot_nt(WRB[...], XN2[r0:r0 + T, :])
                key = score_key(rb(rr[0:8, :]), r0 + lax.broadcasted_iota(jnp.int32, (8, 128), 1))
                RALL[s * NT + c:s * NT + c + 1, :] = key[0:1, :]
            return f
        return [mk(c) for c in range(NT)]

    def top2_prefix():
        k = RALL[...]
        k1 = jnp.max(jnp.maximum(k[0:8], k[8:16]), axis=(0, 1), keepdims=True)
        k = jnp.where(k == k1, jnp.iinfo(jnp.int32).min, k)
        k2 = jnp.max(jnp.maximum(k[0:8], k[8:16]), axis=(0, 1), keepdims=True)
        TOP[0] = jnp.broadcast_to(k1, (8, 128))
        TOP[1] = jnp.broadcast_to(k2, (8, 128))

    def k_pieces(s):
        rows = slice(s * L, (s + 1) * L)
        def mk(g):
            def f():
                k = dot_nn(XN[rows, :], WK[:, g * T:(g + 1) * T])
                set_pace(k)
                KK[g] = k.astype(BF)
                if s < NSEG - 1:
                    pk = phi(k)
                    PK[g] = pk.astype(BF)
                    z = jnp.sum(pk.reshape(L // 8, 8, 128), axis=0)
                    z = jnp.broadcast_to(jnp.sum(z, axis=0, keepdims=True), (8, 128))
                    ZZ[g] = z if s == 0 else ZZ[g] + z
            return f
        return [mk(g) for g in range(G)]

    def k_row_pieces(s):
        def mk(c):
            def f():
                rows = slice(s * L + c * T, s * L + (c + 1) * T)
                k = dot_nn(XN[rows, :], WK[...])
                for g in range(G):
                    kg = k[:, g * T:(g + 1) * T]
                    KK[g, c * T:(c + 1) * T, :] = kg.astype(BF)
                    if s < NSEG - 1:
                        pk = phi(kg)
                        PK[g, c * T:(c + 1) * T, :] = pk.astype(BF)
                        z = jnp.sum(pk.reshape(T // 8, 8, 128), axis=0)
                        ZZ[g] = z if (s == 0 and c == 0) else ZZ[g] + z
            return f
        return [mk(c) for c in range(NT)]

    def q_pieces(s):
        rows = slice(s * L, (s + 1) * L)
        def mk(g):
            def f():
                q = dot_nn(XN[rows, :], WQ[:, g * T:(g + 1) * T])
                set_pace(q)
                QS[g] = (q * QSCALE).astype(BF)
                if s > 0:
                    PQ[g] = phi(q).astype(BF)
            return f
        return [mk(g) for g in range(G)]

    def v_pieces(s):
        def mk(hf, c):
            def f():
                vt = dot_nt(WVT[hf * L:(hf + 1) * L, :], XN[s * L + c * T:s * L + (c + 1) * T, :])
                for gg in range(4):
                    VT[hf * 4 + gg, :, c * T:(c + 1) * T] = vt[gg * T:(gg + 1) * T, :].astype(BF)
            return f
        return [mk(hf, c) for hf in range(2) for c in range(NT)]

    def o_pieces(s):
        rows = slice(s * L, (s + 1) * L)
        def mk(j):
            def f():
                o = jnp.concatenate([OB[g] for g in range(G)], axis=1)
                y = dot_nn(o, WO[:, j * T:(j + 1) * T])
                set_pace(y)
                XM[rows, j * T:(j + 1) * T] = (X[rows, j * T:(j + 1) * T].astype(F32) + rb(y)).astype(BF)
            return f
        return [mk(j) for j in range(G)]

    def o_row_pieces(s):
        def mk(c):
            def f():
                rows = slice(s * L + c * T, s * L + (c + 1) * T)
                o = jnp.concatenate([OB[g, c * T:(c + 1) * T, :] for g in range(G)], axis=1)
                y = dot_nn(o, WO[...])
                XM[rows, :] = (X[rows, :].astype(F32) + rb(y)).astype(BF)
            return f
        return [mk(c) for c in range(NT)]

    def wvt_pieces():
        def mk(i):
            def f():
                for j in range(D // T):
                    WVT[j * T:(j + 1) * T, i * T:(i + 1) * T] = (
                        WV[i * T:(i + 1) * T, j * T:(j + 1) * T].astype(F32).T.astype(BF))
            return f
        return [mk(i) for i in range(D // T)]

    def mem_pieces(s):
        def retrieve(g):
            def f():
                r = dot_nt(AMEM[g], PQ[g])
                for h in range(4):
                    den = r[128 + 4 * h:129 + 4 * h, :] + 1e-6
                    OT[g, DH * h:DH * h + DH, :] = r[DH * h:DH * h + DH, :] * (GATE[4 * g + h][0:1, 0:1] / den)
            return f
        def update(g):
            def f():
                upd = dot_nn(VT[g], PK[g])
                rr = lax.broadcasted_iota(jnp.int32, (128, 128), 0) // DH
                cc = lax.broadcasted_iota(jnp.int32, (128, 128), 1) // DH
                upd = jnp.where(rr == cc, upd, 0.0)
                mt = upd if s == 0 else MT[g] + upd
                if s < NSEG - 2:
                    MT[g] = mt
                AMEM[g, 0:128, :] = mt.astype(BF)
                zr = lax.broadcasted_iota(jnp.int32, (16, 128), 0) // 4
                zc = lax.broadcasted_iota(jnp.int32, (16, 128), 1) // DH
                z = ZZ[g]
                AMEM[g, 128:144, :] = jnp.where(zr == zc, jnp.concatenate([z, z], axis=0), 0.0).astype(BF)
            return f
        ret = [retrieve(g) for g in range(G)] if s > 0 else []
        upd = [update(g) for g in range(G)] if s < NSEG - 1 else []
        return ret, upd

    def p1_steps(g, h, slot, qord='0123'):
        state = {}
        def mk(qt, kt):
            def f():
                if kt == 0:
                    state["qm"] = head_mask(QS[g, qt * T:(qt + 1) * T, :], h)
                    state["m"] = None
                s = dot_nt(KK[g, kt * T:(kt + 1) * T, :], state["qm"])
                if kt == qt:
                    s = jnp.where(rowT <= colT, s, NEG)
                SB[slot, OFF[qt] + kt * T:OFF[qt] + (kt + 1) * T, :] = s
                mt = jnp.max(s.reshape(16, 8, 128), axis=0)
                state["m"] = mt if state["m"] is None else jnp.maximum(state["m"], mt)
                if kt == qt:
                    m = jnp.max(state["m"], axis=0, keepdims=True)
                    MB[slot, qt] = jnp.broadcast_to(m, (8, 128))
            return f
        return [mk(int(qt), kt) for qt in qord for kt in range(int(qt) + 1)]

    def p2_steps(g, h, slot, first_seg, qord='0123'):
        state = {}
        def mk(qt, kt):
            def f():
                if kt == 0:
                    state["m"] = MB[slot, qt]
                    state["l"] = state["acc"] = None
                s = SB[slot, OFF[qt] + kt * T:OFF[qt] + (kt + 1) * T, :]
                p = jnp.exp2(s.reshape(16, 8, 128) - state["m"][None])
                ps = jnp.sum(p, axis=0)
                pv = dot_nn(VT[g, DH * h:DH * h + DH, kt * T:(kt + 1) * T],
                            p.reshape(T, 128).astype(BF))
                state["l"] = ps if state["l"] is None else state["l"] + ps
                state["acc"] = pv if state["acc"] is None else state["acc"] + pv
                if kt == qt:
                    lt = jnp.sum(state["l"], axis=0, keepdims=True)
                    w = (1.0 - GATE[4 * g + h][0:1, :]) / lt
                    res = state["acc"] * w
                    if not first_seg:
                        res = res + OT[g, DH * h:DH * h + DH, qt * T:(qt + 1) * T]
                    OT[g, DH * h:DH * h + DH, qt * T:(qt + 1) * T] = res
            return f
        return [mk(int(qt), kt) for qt in qord for kt in range(int(qt) + 1)]

    def tr_steps(g):
        def mk(qt):
            def f():
                OB[g, qt * T:(qt + 1) * T, :] = OT[g, :, qt * T:(qt + 1) * T].T.astype(BF)
            return f
        return [mk(qt) for qt in range(NT)]

    def attention(s):
        AV = os.environ.get("AV", "12")
        Q1, Q2 = os.environ.get("Q1", "1302"), os.environ.get("Q2", "1302")
        seq_a, seq_b = [], []
        for g in range(G):
            for h in range(4):
                a = p2_steps(g, h, h % 2, s == 0, Q2)
                if h < 3:
                    b = p1_steps(g, h + 1, (h + 1) % 2, Q1)
                elif g < G - 1:
                    b = p1_steps(g + 1, 0, 0, Q1)
                else:
                    b = mem_pieces(s)[1]
                t = tr_steps(g - 1) if (h == 0 and g > 0) else []
                if AV == "21":
                    for i in range(10):
                        a[i]()
                        if i < len(b): b[i]()
                        if i < len(t): t[i]()
                elif AV == "12":
                    for i in range(10):
                        if i < len(b): b[i]()
                        a[i]()
                        if i < len(t): t[i]()
                elif AV == "2211":
                    for i in range(0, 10, 2):
                        a[i](); a[i + 1]()
                        if i < len(b): b[i](); b[i + 1]()
                        if i // 2 < len(t): t[i // 2]()
                elif AV == "ser21":
                    for f in a: f()
                    for f in b: f()
                    for f in t: f()
                elif AV == "ser12":
                    for f in b: f()
                    for f in a: f()
                    for f in t: f()

    def routing_ffn(li):
        t1, t2 = TOP[0], TOP[1]
        k1 = jnp.broadcast_to(jnp.max(t1, axis=0, keepdims=True), (8, 128))
        k2 = jnp.max(jnp.where(t1 == k1, t2, t1), axis=0, keepdims=True)
        k2 = jnp.broadcast_to(k2, (8, 128))
        i1 = jnp.clip(0xFFFF - (k1[0, 0] & 0xFFFF), 0, S - 1)
        i2 = jnp.clip(0xFFFF - (k2[0, 0] & 0xFFFF), 0, S - 1)
        bases = [pl.multiple_of((i >> 4) << 4, 16) for i in (i1, i2)]
        xs = jnp.concatenate([XN2[pl.ds(b, 16), :] for b in bases], axis=0)
        hs = []
        for j in range(NF):
            gg = rb(dot_nn(xs, WG[:, j * T:(j + 1) * T]))
            uu = rb(dot_nn(xs, WU[:, j * T:(j + 1) * T]))
            hs.append((rb(gg * jax.nn.sigmoid(gg)) * uu).astype(BF))
        hh = jnp.concatenate(hs, axis=1)
        ys = [rb(dot_nn(hh, WD[n])) for n in range(D // T)]
        row16 = lax.broadcasted_iota(jnp.int32, (16, D), 0)
        for j, (i, base, kk) in enumerate(zip((i1, i2), bases, (k1, k2))):
            u = kk & jnp.int32(-65536)
            mv = pltpu.bitcast(u ^ ((u >> 31) & 0x7FFF0000), F32)
            rs = rb(jax.nn.sigmoid(mv))
            rs = jnp.concatenate([rs, rs], axis=0)
            upd = jnp.concatenate([rb(yn[16 * j:16 * j + 16, :] * rs) for yn in ys], axis=1)
            blk = XN2[pl.ds(base, 16), :].astype(F32)
            nb = jnp.where(row16 == i - base, rb(blk + upd), blk)
            XN2[pl.ds(base, 16), :] = nb.astype(BF)
            xo = (XM[pl.ds(base, 16), :].astype(F32) + nb).astype(BF)
            X[pl.ds(base, 16), :] = xo
            if li == 0:
                XN[pl.ds(base, 16), :] = layernorm(xo.astype(F32)).astype(BF)
        return bases

    def block_b(li, s):
        first = li == 0
        kp, qp, vp = k_pieces(s), q_pieces(s), v_pieces(s)
        ret = mem_pieces(s)[0]
        p10 = p1_steps(0, 0, 0, os.environ.get("QB", "0123"))
        if s == 0:
            if first:
                if SV in ("0",) or (ONLY and ONLY != "START"):
                    interleave(kp)
                else:
                    cwkc[0].wait()
                    cwv.start()
                    kp[0]()
                    for g in range(1, G):
                        cwkc[g].wait()
                    interleave(kp[1:])
                cwq.wait()
                for c in (cx[1], cwo, cx[2], cx[3]):
                    c.start()
                interleave(qp[:4])
                cwv.wait()
                interleave(qp[4:], wvt_pieces())
                interleave(vp, p10)
                if ONLY != "START":
                    for c in (cx[1], cwo, cx[2], cx[3]):
                        c.wait()
                for c in cwg + cwu + cwd:
                    c.start()
            else:
                interleave(kp + qp)
                interleave(vp, p10)
        else:
            for f in tr_steps(G - 1):
                f()
            interleave(o_pieces(s - 1), ln1_pieces(s))
            ln2, rp = ln2_pieces(s - 1), r_pieces(s - 1)
            q4 = len(ln2) // 4
            interleave(kp[:4], ln2[0:q4])
            interleave(kp[4:], ln2[q4:2 * q4])
            rp[0]()
            interleave(qp[:4], ln2[2 * q4:3 * q4])
            rp[1]()
            interleave(qp[4:], ln2[3 * q4:])
            rp[2]()
            interleave(vp[:2])
            rp[3]()
            if not first and not ONLY:
                cout[s - 1].start()
            BV = os.environ.get("BV", "3")
            if BV == "0":
                interleave(vp[2:], ret + p10)
            elif BV == "1":
                interleave(vp[2:], p10 + ret)
            elif BV == "2":
                interleave(vp[2:], p10, ret)
            elif BV == "3":
                interleave(vp[2:6], ret)
                interleave(vp[6:], p10)
            elif BV == "4":
                interleave(vp[2:])
                interleave(ret + p10)

    def block_t(li):
        first = li == 0
        for f in tr_steps(G - 1):
            f()
        s = NSEG - 1
        TV = os.environ.get("TV", "0")
        top2_prefix()
        op, ln2 = o_row_pieces(s), ln2_pieces(s, int(os.environ.get("TC", "12")), True)
        pace["ch"] = None
        op[0]()
        interleave([op[1]], ln2[0:4])
        interleave([op[2]], ln2[4:8])
        interleave([op[3]], ln2[8:12])
        interleave(ln2[12:16])
        if not first and not ONLY:
            cout[s].start()

    def block_f(li):
        routing_ffn(li)

    def block_a(li, s):
        attention(s)

    def cut(fn):
        lax.fori_loop(0, pl.program_id(0) + 1, lambda i, c: (fn(), c)[1], 0)

    def startup():
        l1 = ln1_pieces(0, chain=False)
        if SV == "0":
            cx[0].wait()
            cwq.start()
            for f in l1: f()
            cwk.wait()
            cwv.start()
        elif SV == "1":
            cx[0].wait()
            cwq.start()
            for f in l1: f()
        elif SV == "2":
            n = len(l1) // NT
            for c in range(NT):
                cx0[c].wait()
                if c == NT - 1:
                    cwq.start()
                for f in l1[c * n:(c + 1) * n]: f()
        elif SV == "3":
            n = len(l1) // NT
            for c in range(NT):
                cx0[c].wait()
                if c == 0:
                    for cc in cwkc: cc.start()
                if c == NT - 1:
                    cwq.start()
                for f in l1[c * n:(c + 1) * n]: f()
        elif SV == "4":
            cx[0].wait()
            for cc in cwkc: cc.start()
            cwq.start()
            for f in l1: f()

    if ONLY == "START":
        startup()
        block_b(0, 0)
        for c in (cx[1], cwo, cx[2], cx[3]) + tuple(cwg + cwu + cwd):
            c.wait()
        return
    if ONLY:
        for item in ONLY.split(";"):
            def run(item=item):
                for name in item.strip("[").split("+"):
                    if name[0] == "T":
                        block_t(int(name[1]))
                        continue
                    if name[0] == "F":
                        block_f(int(name[1]))
                        continue
                    li, s = int(name[1]), int(name[2])
                    (block_a if name[0] == "A" else block_b)(li, s)
            if item.startswith("["):
                cut(run)
            else:
                run()
        cx[0].wait()
        cwk.wait()
        return

    startup()
    for li in range(2):
        first = li == 0
        MV = os.environ.get("MV", "0")
        if MV == "0":
            for s in range(NSEG):
                block_b(li, s)
                cut(lambda: block_a(li, s))
        elif MV == "1":
            block_b(li, 0)
            for s in range(NSEG - 1):
                cut(lambda: (block_a(li, s), block_b(li, s + 1)))
            cut(lambda: block_a(li, NSEG - 1))
        elif MV == "2":
            for s in range(NSEG):
                cut(lambda: (block_b(li, s), block_a(li, s)))
        block_t(li)
        if first:
            for c in cwg + cwu + cwd:
                c.wait()
            interleave(ln1_pieces(0))
        bases = routing_ffn(li)
        if not first:
            for c in cout:
                c.wait()
            p0 = pltpu.make_async_copy(X.at[pl.ds(bases[0], 16), :], out_hbm.at[pl.ds(bases[0], 16), :], sems.at[13])
            p1 = pltpu.make_async_copy(X.at[pl.ds(bases[1], 16), :], out_hbm.at[pl.ds(bases[1], 16), :], sems.at[14])
            p0.start()
            @pl.when(bases[1] != bases[0])
            def _():
                p1.start()
                p1.wait()
            p0.wait()


@jax.jit
def pallas_interleave_layers__memory_aug_infini_attn__moe_arch_mod__prompt_kernel(
    A_x, A_wq, A_wk, A_wv, A_wo, A_beta, B_x, B_w_r, B_w_gate, B_w_up, B_w_down):
    del B_x
    any_spec = pl.BlockSpec(memory_space=pl.ANY)
    vm = pltpu.VMEM
    blk = vm((G, L, 128), BF)
    out = pl.pallas_call(
        kernel,
        out_shape=jax.ShapeDtypeStruct((S, D), BF),
        grid=(1,),
        in_specs=[any_spec, any_spec, any_spec, any_spec, any_spec,
                  pl.BlockSpec((1, H), lambda i: (0, 0)), pl.BlockSpec((8, 128), lambda i: (0, 0)),
                  any_spec, any_spec, any_spec],
        out_specs=any_spec,
        scratch_shapes=[
            vm((S, D), BF), vm((S, D), BF), vm((S, D), BF), vm((S, D), BF),
            vm((D, D), BF), vm((D, D), BF), vm((D, D), BF), vm((D, D), BF), vm((D, D), BF),
            vm((D, F), BF), vm((D, F), BF), vm((D // T, F, T), BF),
            blk, blk, blk, blk, vm((G, 128, L), BF),
            vm((2, 1280, 128), F32), vm((2, NT, 8, 128), F32),
            vm((G, 128, L), F32), blk,
            vm((G, 128, 128), F32), vm((G, 8, 128), F32), vm((G, 144, 128), BF),
            vm((H, 8, 128), F32), vm((8, D), F32), vm((16, D), BF), vm((2, 8, 128), jnp.int32), vm((16, 128), jnp.int32),
            pltpu.SemaphoreType.DMA((29,)),
        ],
        compiler_params=pltpu.CompilerParams(vmem_limit_bytes=110 * 1024 * 1024, flags=FLAGS),
        name="fused",
    )(A_x.reshape(S, D), A_wq, A_wk, A_wv, A_wo, A_beta.reshape(1, H), B_w_r.reshape(8, 128),
      B_w_gate, B_w_up, B_w_down)
    return out.reshape(1, S, D)
```

```python
import jax
import jax.numpy as jnp
import numpy as np
from jax import lax
import jax.experimental.pallas as pl
import jax.experimental.pallas.tpu as pltpu

S, D, F = 2048, 1024, 3584
H, DH = 32, 32
NSEG, L = 4, 512
G, T = 8, 128
NT = L // T
NF = F // T
OFF = (0, 128, 384, 768)
NEG = -1e30
EPS = 1e-5
QSCALE = float(DH ** -0.5 * np.log2(np.e))
BF = jnp.bfloat16
F32 = jnp.float32
import os
LNR = int(os.environ.get('LNR', '32'))
ONLY = os.environ.get('ONLY')
VAR = os.environ.get('VAR', '')
CHAIN = int(os.environ.get('CHAIN', '1'))
FLAGS = {k: True for k in os.environ.get('FLAGS', '').split(',') if k} or None


def dot_nt(a, b):
    return lax.dot_general(a, b, (((1,), (1,)), ((), ())), preferred_element_type=F32)


def dot_nn(a, b):
    return lax.dot_general(a, b, (((1,), (0,)), ((), ())), preferred_element_type=F32)


def rb(x):
    return x.astype(BF).astype(F32)


def layernorm(x, chain=None):
    m = jnp.sum(x, axis=-1, keepdims=True) * (1.0 / D)
    if chain is not None and chain.get("tok") is not None:
        m = jnp.where(chain["never"], chain["tok"], m)
    c = x - m
    v = jnp.sum(c * c, axis=-1, keepdims=True) * (1.0 / D)
    a = rb(rb(v) + EPS)
    y = lax.rsqrt(a)
    s = rb(a * y)
    y = y * (2.0 - s * y)
    if chain is not None:
        chain["tok"] = y
    return c * y


def gate_rows(x, chain):
    if chain is None or chain.get("tok") is None:
        return x
    u = pltpu.bitcast(x, jnp.uint32)
    t = pltpu.bitcast(chain["tok"], jnp.uint32)
    t = jnp.concatenate([t] * (u.shape[1] // 128), axis=1)
    t = jnp.concatenate([t] * (u.shape[0] // 8), axis=0)
    return pltpu.bitcast(jnp.where(chain["never"], t, u), BF)


def phi(t):
    return jnp.where(t > 0, t + 1.0, jnp.exp(t))


def head_mask(x, h):
    u = pltpu.bitcast(x, jnp.uint32)
    lane = lax.broadcasted_iota(jnp.int32, u.shape, 1)
    u = jnp.where((lane >= DH * h) & (lane < DH * h + DH), u, jnp.uint32(0))
    return pltpu.bitcast(u, BF)


def interleave(main, *bgs):
    main = list(main)
    bgs = [list(b) for b in bgs]
    done = [0] * len(bgs)
    n = len(main)
    for i, piece in enumerate(main):
        piece()
        for bi, b in enumerate(bgs):
            upto = (i + 1) * len(b) // n
            while done[bi] < upto:
                b[done[bi]]()
                done[bi] += 1


def kernel(x_hbm, wq_hbm, wk_hbm, wv_hbm, wo_hbm, beta_ref, wr_ref, wg_hbm, wu_hbm, wd_hbm,
           out_hbm,
           X, XM, XN2, XN, WQ, WK, WV, WVT, WO, WG, WU, WD,
           QS, KK, PQ, PK, VT, SB, MB, OT, OB, MT, ZZ, AMEM, GATE, WR, WRB, TOP, RALL, sems):
    def cp(src, dst, i):
        return pltpu.make_async_copy(src, dst, sems.at[i])
    cx = [cp(x_hbm.at[pl.ds(s * L, L), :], X.at[pl.ds(s * L, L), :], s) for s in range(NSEG)]
    cwq, cwk, cwv, cwo = (cp(wq_hbm, WQ, 4), cp(wk_hbm, WK, 5), cp(wv_hbm, WV, 6), cp(wo_hbm, WO, 7))
    cwd = [cp(wd_hbm.at[:, pl.ds(j * T, T)], WD.at[j], 28) for j in range(D // T)]
    cwg = [cp(wg_hbm, WG, 8)]
    cwu = [cp(wu_hbm, WU, 27)]
    cout = [cp(X.at[pl.ds(s * L, L), :], out_hbm.at[pl.ds(s * L, L), :], 9 + s) for s in range(NSEG)]
    SV = os.environ.get("SV", "7")
    cx0 = [cp(x_hbm.at[pl.ds(c * T, T), :], X.at[pl.ds(c * T, T), :], 15 + c) for c in range(NT)]
    cwkc = [cp(wk_hbm.at[:, pl.ds(g * T, T)], WK.at[:, pl.ds(g * T, T)], 19 + g) for g in range(G)]
    if SV == "0":
        cx[0].start()
        cwk.start()
    elif SV == "1":
        cx[0].start()
        for c in cwkc: c.start()
    elif SV == "2":
        for c in cx0: c.start()
        for c in cwkc: c.start()
    elif SV == "3":
        for c in cx0: c.start()
    elif SV == "4":
        cx[0].start()
    elif SV == "7":
        for c in cx0 + cwkc + [cwq, cwv]: c.start()
        if os.environ.get("NOX", "0") == "0":
            for c in (cx[1], cwo, cx[2], cx[3]): c.start()
    elif SV in ("5", "6"):
        NW = int(os.environ.get("NW", "2"))
        for c in cx0: c.start()
        for c in cwkc[:NW]: c.start()

    gate = jax.nn.sigmoid(beta_ref[...].astype(F32))
    for j in range(H):
        GATE[j] = jnp.broadcast_to(gate[:, j:j + 1], (8, 128))
    wr8 = wr_ref[...].astype(F32)
    WR[...] = jnp.concatenate(
        [jnp.broadcast_to(wr8[c:c + 1, :], (8, 128)) for c in range(8)], axis=1)
    WRB[...] = jnp.concatenate(
        [jnp.broadcast_to(wr8[c:c + 1, :], (16, 128)) for c in range(8)], axis=1).astype(BF)
    RALL[...] = jnp.full(RALL.shape, jnp.iinfo(jnp.int32).min, jnp.int32)

    rowT = lax.broadcasted_iota(jnp.int32, (T, T), 0)
    colT = lax.broadcasted_iota(jnp.int32, (T, T), 1)

    never = GATE[0][0:1, 0:1] < -1.0
    PACE = False
    pace = dict(ch=None)
    def set_pace(val):
        if PACE and pace["ch"] is not None:
            pace["ch"]["tok"] = val[0:8, 0:128]
    def new_chain():
        return dict(never=never, tok=None) if CHAIN else None

    def ln1_pieces(s, chain=True):
        ch = new_chain() if chain else None
        pace["ch"] = ch
        def mk(r):
            def f():
                rows = slice(s * L + r * LNR, s * L + (r + 1) * LNR)
                XN[rows, :] = layernorm(X[rows, :].astype(F32), ch).astype(BF)
            return f
        return [mk(r) for r in range(L // LNR)]

    def score_key(sc, tok):
        u = pltpu.bitcast(sc, jnp.int32)
        return (u ^ ((u >> 31) & 0x7FFF0000)) | (0xFFFF - tok)

    def ln2_pieces(s, chain_upto=99, route=False):
        ch = new_chain()
        nrg = LNR // 8
        def mk(r):
            def f():
                if r >= chain_upto:
                    ch["tok"] = None
                r0 = s * L + r * LNR
                rows = slice(r0, r0 + LNR)
                xm = XM[rows, :].astype(F32)
                xn2 = layernorm(xm, ch).astype(BF)
                XN2[rows, :] = xn2
                xf = xn2.astype(F32)
                X[rows, :] = (xm + xf).astype(BF)
                if route:
                    prod = xf.reshape(nrg, 8, D) * WR[...][None]
                    sc = rb(jnp.sum(prod, axis=-1, keepdims=True))
                    sc = jnp.broadcast_to(sc, (nrg, 8, 128)).reshape(LNR, 128)
                    key = score_key(sc, r0 + lax.broadcasted_iota(jnp.int32, (LNR, 128), 0))
                    t1, t2 = TOP[0], TOP[1]
                    for j in range(nrg):
                        kj = key[8 * j:8 * j + 8]
                        t2 = jnp.maximum(t2, jnp.minimum(t1, kj))
                        t1 = jnp.maximum(t1, kj)
                    TOP[0] = t1
                    TOP[1] = t2
            return f
        return [mk(r) for r in range(L // LNR)]

    def r_pieces(s):
        def mk(c):
            def f():
                r0 = s * L + c * T
                rr = dot_nt(WRB[...], XN2[r0:r0 + T, :])
                key = score_key(rb(rr[0:8, :]), r0 + lax.broadcasted_iota(jnp.int32, (8, 128), 1))
                RALL[s * NT + c:s * NT + c + 1, :] = key[0:1, :]
            return f
        return [mk(c) for c in range(NT)]

    def top2_prefix():
        k = RALL[...]
        k1 = jnp.max(jnp.maximum(k[0:8], k[8:16]), axis=(0, 1), keepdims=True)
        k = jnp.where(k == k1, jnp.iinfo(jnp.int32).min, k)
        k2 = jnp.max(jnp.maximum(k[0:8], k[8:16]), axis=(0, 1), keepdims=True)
        TOP[0] = jnp.broadcast_to(k1, (8, 128))
        TOP[1] = jnp.broadcast_to(k2, (8, 128))

    def k_pieces(s):
        rows = slice(s * L, (s + 1) * L)
        def mk(g):
            def f():
                k = dot_nn(XN[rows, :], WK[:, g * T:(g + 1) * T])
                set_pace(k)
                KK[g] = k.astype(BF)
                if s < NSEG - 1:
                    pk = phi(k)
                    PK[g] = pk.astype(BF)
                    z = jnp.sum(pk.reshape(L // 8, 8, 128), axis=0)
                    z = jnp.broadcast_to(jnp.sum(z, axis=0, keepdims=True), (8, 128))
                    ZZ[g] = z if s == 0 else ZZ[g] + z
            return f
        return [mk(g) for g in range(G)]

    def k_row_pieces(s):
        def mk(c):
            def f():
                rows = slice(s * L + c * T, s * L + (c + 1) * T)
                k = dot_nn(XN[rows, :], WK[...])
                for g in range(G):
                    kg = k[:, g * T:(g + 1) * T]
                    KK[g, c * T:(c + 1) * T, :] = kg.astype(BF)
                    if s < NSEG - 1:
                        pk = phi(kg)
                        PK[g, c * T:(c + 1) * T, :] = pk.astype(BF)
                        z = jnp.sum(pk.reshape(T // 8, 8, 128), axis=0)
                        ZZ[g] = z if (s == 0 and c == 0) else ZZ[g] + z
            return f
        return [mk(c) for c in range(NT)]

    def q_pieces(s):
        rows = slice(s * L, (s + 1) * L)
        def mk(g):
            def f():
                q = dot_nn(XN[rows, :], WQ[:, g * T:(g + 1) * T])
                set_pace(q)
                QS[g] = (q * QSCALE).astype(BF)
                if s > 0:
                    PQ[g] = phi(q).astype(BF)
            return f
        return [mk(g) for g in range(G)]

    def v_pieces(s):
        def mk(hf, c):
            def f():
                vt = dot_nt(WVT[hf * L:(hf + 1) * L, :], XN[s * L + c * T:s * L + (c + 1) * T, :])
                for gg in range(4):
                    VT[hf * 4 + gg, :, c * T:(c + 1) * T] = vt[gg * T:(gg + 1) * T, :].astype(BF)
            return f
        return [mk(hf, c) for hf in range(2) for c in range(NT)]

    def o_pieces(s):
        rows = slice(s * L, (s + 1) * L)
        def mk(j):
            def f():
                o = jnp.concatenate([OB[g] for g in range(G)], axis=1)
                y = dot_nn(o, WO[:, j * T:(j + 1) * T])
                set_pace(y)
                XM[rows, j * T:(j + 1) * T] = (X[rows, j * T:(j + 1) * T].astype(F32) + rb(y)).astype(BF)
            return f
        return [mk(j) for j in range(G)]

    def o_row_pieces(s):
        def mk(c):
            def f():
                rows = slice(s * L + c * T, s * L + (c + 1) * T)
                o = jnp.concatenate([OB[g, c * T:(c + 1) * T, :] for g in range(G)], axis=1)
                y = dot_nn(o, WO[...])
                XM[rows, :] = (X[rows, :].astype(F32) + rb(y)).astype(BF)
            return f
        return [mk(c) for c in range(NT)]

    def wvt_pieces():
        def mk(i):
            def f():
                for j in range(D // T):
                    WVT[j * T:(j + 1) * T, i * T:(i + 1) * T] = (
                        WV[i * T:(i + 1) * T, j * T:(j + 1) * T].astype(F32).T.astype(BF))
            return f
        return [mk(i) for i in range(D // T)]

    def mem_pieces(s):
        def retrieve(g):
            def f():
                r = dot_nt(AMEM[g], PQ[g])
                for h in range(4):
                    den = r[128 + 4 * h:129 + 4 * h, :] + 1e-6
                    OT[g, DH * h:DH * h + DH, :] = r[DH * h:DH * h + DH, :] * (GATE[4 * g + h][0:1, 0:1] / den)
            return f
        def update(g):
            def f():
                upd = dot_nn(VT[g], PK[g])
                rr = lax.broadcasted_iota(jnp.int32, (128, 128), 0) // DH
                cc = lax.broadcasted_iota(jnp.int32, (128, 128), 1) // DH
                upd = jnp.where(rr == cc, upd, 0.0)
                mt = upd if s == 0 else MT[g] + upd
                if s < NSEG - 2:
                    MT[g] = mt
                AMEM[g, 0:128, :] = mt.astype(BF)
                zr = lax.broadcasted_iota(jnp.int32, (16, 128), 0) // 4
                zc = lax.broadcasted_iota(jnp.int32, (16, 128), 1) // DH
                z = ZZ[g]
                AMEM[g, 128:144, :] = jnp.where(zr == zc, jnp.concatenate([z, z], axis=0), 0.0).astype(BF)
            return f
        ret = [retrieve(g) for g in range(G)] if s > 0 else []
        upd = [update(g) for g in range(G)] if s < NSEG - 1 else []
        return ret, upd

    def p1_steps(g, h, slot, qord='0123'):
        state = {}
        def mk(qt, kt):
            def f():
                if kt == 0:
                    state["qm"] = head_mask(QS[g, qt * T:(qt + 1) * T, :], h)
                    state["m"] = None
                s = dot_nt(KK[g, kt * T:(kt + 1) * T, :], state["qm"])
                if kt == qt:
                    s = jnp.where(rowT <= colT, s, NEG)
                SB[slot, OFF[qt] + kt * T:OFF[qt] + (kt + 1) * T, :] = s
                mt = jnp.max(s.reshape(16, 8, 128), axis=0)
                state["m"] = mt if state["m"] is None else jnp.maximum(state["m"], mt)
                if kt == qt:
                    m = jnp.max(state["m"], axis=0, keepdims=True)
                    MB[slot, qt] = jnp.broadcast_to(m, (8, 128))
            return f
        return [mk(int(qt), kt) for qt in qord for kt in range(int(qt) + 1)]

    def p2_steps(g, h, slot, first_seg, qord='0123'):
        state = {}
        def mk(qt, kt):
            def f():
                if kt == 0:
                    state["m"] = MB[slot, qt]
                    state["l"] = state["acc"] = None
                s = SB[slot, OFF[qt] + kt * T:OFF[qt] + (kt + 1) * T, :]
                p = jnp.exp2(s.reshape(16, 8, 128) - state["m"][None])
                ps = jnp.sum(p, axis=0)
                pv = dot_nn(VT[g, DH * h:DH * h + DH, kt * T:(kt + 1) * T],
                            p.reshape(T, 128).astype(BF))
                state["l"] = ps if state["l"] is None else state["l"] + ps
                state["acc"] = pv if state["acc"] is None else state["acc"] + pv
                if kt == qt:
                    lt = jnp.sum(state["l"], axis=0, keepdims=True)
                    w = (1.0 - GATE[4 * g + h][0:1, :]) / lt
                    res = state["acc"] * w
                    if not first_seg:
                        res = res + OT[g, DH * h:DH * h + DH, qt * T:(qt + 1) * T]
                    OT[g, DH * h:DH * h + DH, qt * T:(qt + 1) * T] = res
            return f
        return [mk(int(qt), kt) for qt in qord for kt in range(int(qt) + 1)]

    def tr_steps(g):
        def mk(qt):
            def f():
                OB[g, qt * T:(qt + 1) * T, :] = OT[g, :, qt * T:(qt + 1) * T].T.astype(BF)
            return f
        return [mk(qt) for qt in range(NT)]

    def attention(s):
        AV = os.environ.get("AV", "12")
        Q1, Q2 = os.environ.get("Q1", "1302"), os.environ.get("Q2", "1302")
        seq_a, seq_b = [], []
        for g in range(G):
            for h in range(4):
                a = p2_steps(g, h, h % 2, s == 0, Q2)
                if h < 3:
                    b = p1_steps(g, h + 1, (h + 1) % 2, Q1)
                elif g < G - 1:
                    b = p1_steps(g + 1, 0, 0, Q1)
                else:
                    b = mem_pieces(s)[1]
                t = tr_steps(g - 1) if (h == 0 and g > 0) else []
                if AV == "21":
                    for i in range(10):
                        a[i]()
                        if i < len(b): b[i]()
                        if i < len(t): t[i]()
                elif AV == "12":
                    for i in range(10):
                        if i < len(b): b[i]()
                        a[i]()
                        if i < len(t): t[i]()
                elif AV == "2211":
                    for i in range(0, 10, 2):
                        a[i](); a[i + 1]()
                        if i < len(b): b[i](); b[i + 1]()
                        if i // 2 < len(t): t[i // 2]()
                elif AV == "ser21":
                    for f in a: f()
                    for f in b: f()
                    for f in t: f()
                elif AV == "ser12":
                    for f in b: f()
                    for f in a: f()
                    for f in t: f()

    def routing_ffn(li):
        t1, t2 = TOP[0], TOP[1]
        k1 = jnp.broadcast_to(jnp.max(t1, axis=0, keepdims=True), (8, 128))
        k2 = jnp.max(jnp.where(t1 == k1, t2, t1), axis=0, keepdims=True)
        k2 = jnp.broadcast_to(k2, (8, 128))
        i1 = jnp.clip(0xFFFF - (k1[0, 0] & 0xFFFF), 0, S - 1)
        i2 = jnp.clip(0xFFFF - (k2[0, 0] & 0xFFFF), 0, S - 1)
        bases = [pl.multiple_of((i >> 4) << 4, 16) for i in (i1, i2)]
        xs = jnp.concatenate([XN2[pl.ds(b, 16), :] for b in bases], axis=0)
        hs = []
        for j in range(NF):
            gg = rb(dot_nn(xs, WG[:, j * T:(j + 1) * T]))
            uu = rb(dot_nn(xs, WU[:, j * T:(j + 1) * T]))
            hs.append((rb(gg * jax.nn.sigmoid(gg)) * uu).astype(BF))
        hh = jnp.concatenate(hs, axis=1)
        ys = [rb(dot_nn(hh, WD[n])) for n in range(D // T)]
        row16 = lax.broadcasted_iota(jnp.int32, (16, D), 0)
        for j, (i, base, kk) in enumerate(zip((i1, i2), bases, (k1, k2))):
            u = kk & jnp.int32(-65536)
            mv = pltpu.bitcast(u ^ ((u >> 31) & 0x7FFF0000), F32)
            rs = rb(jax.nn.sigmoid(mv))
            rs = jnp.concatenate([rs, rs], axis=0)
            upd = jnp.concatenate([rb(yn[16 * j:16 * j + 16, :] * rs) for yn in ys], axis=1)
            blk = XN2[pl.ds(base, 16), :].astype(F32)
            nb = jnp.where(row16 == i - base, rb(blk + upd), blk)
            XN2[pl.ds(base, 16), :] = nb.astype(BF)
            xo = (XM[pl.ds(base, 16), :].astype(F32) + nb).astype(BF)
            X[pl.ds(base, 16), :] = xo
            if li == 0:
                XN[pl.ds(base, 16), :] = layernorm(xo.astype(F32)).astype(BF)
        return bases

    def block_b(li, s):
        first = li == 0
        kp, qp, vp = k_pieces(s), q_pieces(s), v_pieces(s)
        ret = mem_pieces(s)[0]
        p10 = p1_steps(0, 0, 0, os.environ.get("QB", "0123"))
        if s == 0:
            if first:
                if SV in ("0",) or (ONLY and ONLY != "START"):
                    interleave(kp)
                    cwq.wait()
                    interleave(qp[:4])
                    cwv.wait()
                elif SV == "7":
                    groups = [[int(ch) for ch in grp] for grp in os.environ.get("WG", "0,1,23,4567").split(",")]
                    for grp in groups:
                        for g in grp: cwkc[g].wait()
                        for g in grp: kp[g]()
                    cwq.wait()
                    interleave(qp[:4])
                elif SV in ("5", "6"):
                    for g in range(NW):
                        cwkc[g].wait()
                    interleave(kp[:NW])
                    for g in range(NW, G):
                        cwkc[g].wait()
                    cwq.start()
                    interleave(kp[NW:])
                    cwq.wait()
                    cwv.start()
                    interleave(qp[:4])
                    cwv.wait()
                    if os.environ.get("NOX", "0") == "0":
                        for c in (cx[1], cwo, cx[2], cx[3]):
                            c.start()
                else:
                    cwkc[0].wait()
                    cwv.start()
                    kp[0]()
                    for g in range(1, G):
                        cwkc[g].wait()
                    interleave(kp[1:])
                    cwq.wait()
                    if os.environ.get("NOX", "0") == "0":
                        for c in (cx[1], cwo, cx[2], cx[3]):
                            c.start()
                    interleave(qp[:4])
                    cwv.wait()
                if SV == "7" and (ONLY in (None, "START")):
                    qp[4]()
                    cwv.wait()
                    interleave(qp[5:], wvt_pieces())
                else:
                    interleave(qp[4:], wvt_pieces())
                interleave(vp, p10)
                if ONLY == "START" and os.environ.get("NOF", "0") == "0":
                    for c in cwg + cwu + cwd:
                        c.start()
            else:
                interleave(kp + qp)
                interleave(vp, p10)
        else:
            for f in tr_steps(G - 1):
                f()
            interleave(o_pieces(s - 1), ln1_pieces(s))
            ln2, rp = ln2_pieces(s - 1), r_pieces(s - 1)
            q4 = len(ln2) // 4
            interleave(kp[:4], ln2[0:q4])
            interleave(kp[4:], ln2[q4:2 * q4])
            rp[0]()
            interleave(qp[:4], ln2[2 * q4:3 * q4])
            rp[1]()
            interleave(qp[4:], ln2[3 * q4:])
            rp[2]()
            interleave(vp[:2])
            rp[3]()
            if not first and not ONLY:
                cout[s - 1].start()
            BV = os.environ.get("BV", "3")
            if BV == "0":
                interleave(vp[2:], ret + p10)
            elif BV == "1":
                interleave(vp[2:], p10 + ret)
            elif BV == "2":
                interleave(vp[2:], p10, ret)
            elif BV == "3":
                interleave(vp[2:6], ret)
                interleave(vp[6:], p10)
            elif BV == "4":
                interleave(vp[2:])
                interleave(ret + p10)

    def block_t(li):
        first = li == 0
        for f in tr_steps(G - 1):
            f()
        s = NSEG - 1
        TV = os.environ.get("TV", "0")
        top2_prefix()
        op, ln2 = o_row_pieces(s), ln2_pieces(s, int(os.environ.get("TC", "12")), True)
        pace["ch"] = None
        op[0]()
        interleave([op[1]], ln2[0:4])
        interleave([op[2]], ln2[4:8])
        interleave([op[3]], ln2[8:12])
        interleave(ln2[12:16])
        if not first and not ONLY:
            cout[s].start()

    def block_f(li):
        routing_ffn(li)

    def block_a(li, s):
        attention(s)
        if ONLY:
            return
        if li == 0 and s == 0:
            for c in (cx[1], cwo, cx[2], cx[3]):
                c.wait()
            for c in cwg + cwu + cwd:
                c.start()
        if li == 0 and s == NSEG - 1:
            for c in cwg + cwu + cwd:
                c.wait()
        if li == 1 and s == NSEG - 1:
            for c in cout[:NSEG - 1]:
                c.wait()

    def cut(fn):
        lax.fori_loop(0, pl.program_id(0) + 1, lambda i, c: (fn(), c)[1], 0)

    def startup():
        l1 = ln1_pieces(0, chain=False)
        if SV == "0":
            cx[0].wait()
            cwq.start()
            for f in l1: f()
            cwk.wait()
            cwv.start()
        elif SV == "1":
            cx[0].wait()
            cwq.start()
            for f in l1: f()
        elif SV == "2":
            n = len(l1) // NT
            for c in range(NT):
                cx0[c].wait()
                if c == NT - 1:
                    cwq.start()
                for f in l1[c * n:(c + 1) * n]: f()
        elif SV == "3":
            n = len(l1) // NT
            for c in range(NT):
                cx0[c].wait()
                if c == 0:
                    for cc in cwkc: cc.start()
                if c == NT - 1:
                    cwq.start()
                for f in l1[c * n:(c + 1) * n]: f()
        elif SV == "7":
            n = len(l1) // NT
            for c in range(NT):
                cx0[c].wait()
                for f in l1[c * n:(c + 1) * n]: f()
        elif SV in ("5", "6"):
            n = len(l1) // NT
            for c in range(NT):
                cx0[c].wait()
                if c == (NT - 1 if SV == "5" else 1):
                    for cc in cwkc[NW:]: cc.start()
                for f in l1[c * n:(c + 1) * n]: f()
        elif SV == "4":
            cx[0].wait()
            for cc in cwkc: cc.start()
            cwq.start()
            for f in l1: f()

    if ONLY == "START":
        startup()
        block_b(0, 0)
        if os.environ.get("NOX", "0") == "0":
            for c in (cx[1], cwo, cx[2], cx[3]):
                c.wait()
        if os.environ.get("NOF", "0") == "0":
            for c in tuple(cwg + cwu + cwd):
                c.wait()
        return
    if ONLY:
        for item in ONLY.split(";"):
            def run(item=item):
                for name in item.strip("[").split("+"):
                    if name[0] == "T":
                        block_t(int(name[1]))
                        continue
                    if name[0] == "F":
                        block_f(int(name[1]))
                        continue
                    li, s = int(name[1]), int(name[2])
                    (block_a if name[0] == "A" else block_b)(li, s)
            if item.startswith("["):
                cut(run)
            else:
                run()
        cx[0].wait()
        cwk.wait()
        return

    startup()
    for li in range(2):
        first = li == 0
        MV = os.environ.get("MV", "0")
        if MV == "0":
            for s in range(NSEG):
                block_b(li, s)
                cut(lambda: block_a(li, s))
        elif MV == "1":
            block_b(li, 0)
            for s in range(NSEG - 1):
                cut(lambda: (block_a(li, s), block_b(li, s + 1)))
            cut(lambda: block_a(li, NSEG - 1))
        elif MV == "2":
            for s in range(NSEG):
                cut(lambda: (block_b(li, s), block_a(li, s)))
        block_t(li)
        if first:
            interleave(ln1_pieces(0))
        bases = routing_ffn(li)
        if not first:
            cout[NSEG - 1].wait()
            p0 = pltpu.make_async_copy(X.at[pl.ds(bases[0], 16), :], out_hbm.at[pl.ds(bases[0], 16), :], sems.at[13])
            p1 = pltpu.make_async_copy(X.at[pl.ds(bases[1], 16), :], out_hbm.at[pl.ds(bases[1], 16), :], sems.at[14])
            p0.start()
            @pl.when(bases[1] != bases[0])
            def _():
                p1.start()
                p1.wait()
            p0.wait()


@jax.jit
def pallas_interleave_layers__memory_aug_infini_attn__moe_arch_mod__prompt_kernel(
    A_x, A_wq, A_wk, A_wv, A_wo, A_beta, B_x, B_w_r, B_w_gate, B_w_up, B_w_down):
    del B_x
    any_spec = pl.BlockSpec(memory_space=pl.ANY)
    vm = pltpu.VMEM
    blk = vm((G, L, 128), BF)
    out = pl.pallas_call(
        kernel,
        out_shape=jax.ShapeDtypeStruct((S, D), BF),
        grid=(1,),
        in_specs=[any_spec, any_spec, any_spec, any_spec, any_spec,
                  pl.BlockSpec((1, H), lambda i: (0, 0)), pl.BlockSpec((8, 128), lambda i: (0, 0)),
                  any_spec, any_spec, any_spec],
        out_specs=any_spec,
        scratch_shapes=[
            vm((S, D), BF), vm((S, D), BF), vm((S, D), BF), vm((S, D), BF),
            vm((D, D), BF), vm((D, D), BF), vm((D, D), BF), vm((D, D), BF), vm((D, D), BF),
            vm((D, F), BF), vm((D, F), BF), vm((D // T, F, T), BF),
            blk, blk, blk, blk, vm((G, 128, L), BF),
            vm((2, 1280, 128), F32), vm((2, NT, 8, 128), F32),
            vm((G, 128, L), F32), blk,
            vm((G, 128, 128), F32), vm((G, 8, 128), F32), vm((G, 144, 128), BF),
            vm((H, 8, 128), F32), vm((8, D), F32), vm((16, D), BF), vm((2, 8, 128), jnp.int32), vm((16, 128), jnp.int32),
            pltpu.SemaphoreType.DMA((29,)),
        ],
        compiler_params=pltpu.CompilerParams(vmem_limit_bytes=110 * 1024 * 1024, flags=FLAGS),
        name="fused",
    )(A_x.reshape(S, D), A_wq, A_wk, A_wv, A_wo, A_beta.reshape(1, H), B_w_r.reshape(8, 128),
      B_w_gate, B_w_up, B_w_down)
    return out.reshape(1, S, D)
```

```python
import jax
import jax.numpy as jnp
import numpy as np
from jax import lax
import jax.experimental.pallas as pl
import jax.experimental.pallas.tpu as pltpu

S, D, F = 2048, 1024, 3584
H, DH = 32, 32
NSEG, L = 4, 512
G, T = 8, 128
NT = L // T
NF = F // T
OFF = (0, 128, 384, 768)
NEG = -1e30
EPS = 1e-5
QSCALE = float(DH ** -0.5 * np.log2(np.e))
BF = jnp.bfloat16
F32 = jnp.float32
I32 = jnp.int32
IMIN = -2 ** 31
LNR = 32
QORD = "1302"


def dot_nt(a, b):
    return lax.dot_general(a, b, (((1,), (1,)), ((), ())), preferred_element_type=F32)


def dot_nn(a, b):
    return lax.dot_general(a, b, (((1,), (0,)), ((), ())), preferred_element_type=F32)


def rb(x):
    return x.astype(BF).astype(F32)


def layernorm(x, chain=None):
    m = jnp.sum(x, axis=-1, keepdims=True) * (1.0 / D)
    if chain is not None and chain["tok"] is not None:
        m = jnp.where(chain["never"], chain["tok"], m)
    c = x - m
    v = jnp.sum(c * c, axis=-1, keepdims=True) * (1.0 / D)
    a = rb(rb(v) + EPS)
    y = lax.rsqrt(a)
    s = rb(a * y)
    y = y * (2.0 - s * y)
    if chain is not None:
        chain["tok"] = y
    return c * y


def phi(t):
    return jnp.where(t > 0, t + 1.0, jnp.exp(t))


def head_mask(x, h):
    u = pltpu.bitcast(x, jnp.uint32)
    lane = lax.broadcasted_iota(I32, u.shape, 1)
    u = jnp.where((lane >= DH * h) & (lane < DH * h + DH), u, jnp.uint32(0))
    return pltpu.bitcast(u, BF)


def score_key(sc, tok):
    u = pltpu.bitcast(sc, I32)
    return (u ^ ((u >> 31) & 0x7FFF0000)) | (0xFFFF - tok)


def interleave(main, *bgs):
    done = [0] * len(bgs)
    n = len(main)
    for i, piece in enumerate(main):
        piece()
        for bi, b in enumerate(bgs):
            upto = (i + 1) * len(b) // n
            while done[bi] < upto:
                b[done[bi]]()
                done[bi] += 1


def kernel(x_hbm, wq_hbm, wk_hbm, wv_hbm, wo_hbm, beta_ref, wr_ref, wg_hbm, wu_hbm, wd_hbm,
           out_hbm,
           X, XM, XN2, XN, WQ, WK, WV, WVT, WO, WG, WU, WD,
           QS, KK, PQ, PK, VT, SB, MB, OT, OB, MT, ZZ, AMEM, GATE, WR, WRB, TOP, RALL, sems):

    def cp(src, dst, i):
        return pltpu.make_async_copy(src, dst, sems.at[i])
    cx0 = [cp(x_hbm.at[pl.ds(c * T, T), :], X.at[pl.ds(c * T, T), :], c) for c in range(NT)]
    cx = [cp(x_hbm.at[pl.ds(s * L, L), :], X.at[pl.ds(s * L, L), :], 3 + s) for s in range(1, NSEG)]
    cwk = [cp(wk_hbm.at[:, pl.ds(g * T, T)], WK.at[:, pl.ds(g * T, T)], 7 + g) for g in range(G)]
    cwq, cwv, cwo = cp(wq_hbm, WQ, 15), cp(wv_hbm, WV, 16), cp(wo_hbm, WO, 17)
    cffn = ([cp(wg_hbm, WG, 18), cp(wu_hbm, WU, 19)]
            + [cp(wd_hbm.at[:, pl.ds(j * T, T)], WD.at[j], 20 + j) for j in range(D // T)])
    cout = [cp(X.at[pl.ds(s * L, L), :], out_hbm.at[pl.ds(s * L, L), :], 28 + s) for s in range(NSEG)]

    for c in cx0 + cwk + [cwq, cwv, cx[0], cwo, cx[1], cx[2]]:
        c.start()

    gate = jax.nn.sigmoid(beta_ref[...].astype(F32))
    for j in range(H):
        GATE[j] = jnp.broadcast_to(gate[:, j:j + 1], (8, 128))
    wr8 = wr_ref[...].astype(F32)
    WR[...] = jnp.concatenate(
        [jnp.broadcast_to(wr8[c:c + 1, :], (8, 128)) for c in range(8)], axis=1)
    WRB[...] = jnp.concatenate(
        [jnp.broadcast_to(wr8[c:c + 1, :], (16, 128)) for c in range(8)], axis=1).astype(BF)
    RALL[...] = jnp.full(RALL.shape, IMIN, I32)

    rowT = lax.broadcasted_iota(I32, (T, T), 0)
    colT = lax.broadcasted_iota(I32, (T, T), 1)
    never = GATE[0][0:1, 0:1] < -1.0

    def new_chain():
        return dict(never=never, tok=None)

    def ln1_pieces(s, chain=True):
        ch = new_chain() if chain else None
        def mk(r):
            def f():
                rr = slice(s * L + r * LNR, s * L + (r + 1) * LNR)
                XN[rr, :] = layernorm(X[rr, :].astype(F32), ch).astype(BF)
            return f
        return [mk(r) for r in range(L // LNR)]

    def ln2_pieces(s, chain_upto=L // LNR, route=False):
        ch = new_chain()
        nrg = LNR // 8
        def mk(r):
            def f():
                if r >= chain_upto:
                    ch["tok"] = None
                r0 = s * L + r * LNR
                rr = slice(r0, r0 + LNR)
                xm = XM[rr, :].astype(F32)
                xn2 = layernorm(xm, ch).astype(BF)
                XN2[rr, :] = xn2
                xf = xn2.astype(F32)
                X[rr, :] = (xm + xf).astype(BF)
                if route:
                    prod = xf.reshape(nrg, 8, D) * WR[...][None]
                    sc = rb(jnp.sum(prod, axis=-1, keepdims=True))
                    sc = jnp.broadcast_to(sc, (nrg, 8, 128)).reshape(LNR, 128)
                    key = score_key(sc, r0 + lax.broadcasted_iota(I32, (LNR, 128), 0))
                    t1, t2 = TOP[0], TOP[1]
                    for j in range(nrg):
                        kj = key[8 * j:8 * j + 8]
                        t2 = jnp.maximum(t2, jnp.minimum(t1, kj))
                        t1 = jnp.maximum(t1, kj)
                    TOP[0] = t1
                    TOP[1] = t2
            return f
        return [mk(r) for r in range(L // LNR)]

    def r_pieces(s):
        def mk(c):
            def f():
                r0 = s * L + c * T
                rr = dot_nt(WRB[...], XN2[r0:r0 + T, :])
                key = score_key(rb(rr[0:8, :]), r0 + lax.broadcasted_iota(I32, (8, 128), 1))
                RALL[s * NT + c:s * NT + c + 1, :] = key[0:1, :]
            return f
        return [mk(c) for c in range(NT)]

    def top2_prefix():
        k = RALL[...]
        k1 = jnp.max(jnp.maximum(k[0:8], k[8:16]), axis=(0, 1), keepdims=True)
        k = jnp.where(k == k1, IMIN, k)
        k2 = jnp.max(jnp.maximum(k[0:8], k[8:16]), axis=(0, 1), keepdims=True)
        TOP[0] = jnp.broadcast_to(k1, (8, 128))
        TOP[1] = jnp.broadcast_to(k2, (8, 128))

    def k_pieces(s):
        rr = slice(s * L, (s + 1) * L)
        def mk(g):
            def f():
                k = dot_nn(XN[rr, :], WK[:, g * T:(g + 1) * T])
                KK[g] = k.astype(BF)
                if s < NSEG - 1:
                    pk = phi(k)
                    PK[g] = pk.astype(BF)
                    z = jnp.sum(pk.reshape(L // 8, 8, 128), axis=0)
                    z = jnp.broadcast_to(jnp.sum(z, axis=0, keepdims=True), (8, 128))
                    ZZ[g] = z if s == 0 else ZZ[g] + z
            return f
        return [mk(g) for g in range(G)]

    def q_pieces(s):
        rr = slice(s * L, (s + 1) * L)
        def mk(g):
            def f():
                q = dot_nn(XN[rr, :], WQ[:, g * T:(g + 1) * T])
                QS[g] = (q * QSCALE).astype(BF)
                if s > 0:
                    PQ[g] = phi(q).astype(BF)
            return f
        return [mk(g) for g in range(G)]

    def v_pieces(s):
        def mk(hf, c):
            def f():
                vt = dot_nt(WVT[hf * L:(hf + 1) * L, :], XN[s * L + c * T:s * L + (c + 1) * T, :])
                for gg in range(4):
                    VT[hf * 4 + gg, :, c * T:(c + 1) * T] = vt[gg * T:(gg + 1) * T, :].astype(BF)
            return f
        return [mk(hf, c) for hf in range(2) for c in range(NT)]

    def o_pieces(s):
        rr = slice(s * L, (s + 1) * L)
        def mk(j):
            def f():
                o = jnp.concatenate([OB[g] for g in range(G)], axis=1)
                y = dot_nn(o, WO[:, j * T:(j + 1) * T])
                XM[rr, j * T:(j + 1) * T] = (X[rr, j * T:(j + 1) * T].astype(F32) + rb(y)).astype(BF)
            return f
        return [mk(j) for j in range(G)]

    def o_row_pieces(s):
        def mk(c):
            def f():
                rr = slice(s * L + c * T, s * L + (c + 1) * T)
                o = jnp.concatenate([OB[g, c * T:(c + 1) * T, :] for g in range(G)], axis=1)
                y = dot_nn(o, WO[...])
                XM[rr, :] = (X[rr, :].astype(F32) + rb(y)).astype(BF)
            return f
        return [mk(c) for c in range(NT)]

    def wvt_pieces():
        def mk(i):
            def f():
                for j in range(D // T):
                    WVT[j * T:(j + 1) * T, i * T:(i + 1) * T] = (
                        WV[i * T:(i + 1) * T, j * T:(j + 1) * T].astype(F32).T.astype(BF))
            return f
        return [mk(i) for i in range(D // T)]

    def retrieve_pieces():
        def mk(g):
            def f():
                r = dot_nt(AMEM[g], PQ[g])
                for h in range(4):
                    den = r[128 + 4 * h:129 + 4 * h, :] + 1e-6
                    OT[g, DH * h:DH * h + DH, :] = (
                        r[DH * h:DH * h + DH, :] * (GATE[4 * g + h][0:1, 0:1] / den))
            return f
        return [mk(g) for g in range(G)]

    def update_pieces(s):
        def mk(g):
            def f():
                upd = dot_nn(VT[g], PK[g])
                rr = lax.broadcasted_iota(I32, (128, 128), 0) // DH
                cc = lax.broadcasted_iota(I32, (128, 128), 1) // DH
                upd = jnp.where(rr == cc, upd, 0.0)
                mt = upd if s == 0 else MT[g] + upd
                if s < NSEG - 2:
                    MT[g] = mt
                AMEM[g, 0:128, :] = mt.astype(BF)
                zr = lax.broadcasted_iota(I32, (16, 128), 0) // 4
                zc = lax.broadcasted_iota(I32, (16, 128), 1) // DH
                z = ZZ[g]
                AMEM[g, 128:144, :] = jnp.where(zr == zc, jnp.concatenate([z, z], axis=0), 0.0).astype(BF)
            return f
        return [mk(g) for g in range(G)]

    def p1_steps(g, h, slot, qord):
        state = {}
        def mk(qt, kt):
            def f():
                if kt == 0:
                    state["qm"] = head_mask(QS[g, qt * T:(qt + 1) * T, :], h)
                    state["m"] = None
                s = dot_nt(KK[g, kt * T:(kt + 1) * T, :], state["qm"])
                if kt == qt:
                    s = jnp.where(rowT <= colT, s, NEG)
                SB[slot, OFF[qt] + kt * T:OFF[qt] + (kt + 1) * T, :] = s
                mt = jnp.max(s.reshape(16, 8, 128), axis=0)
                state["m"] = mt if state["m"] is None else jnp.maximum(state["m"], mt)
                if kt == qt:
                    m = jnp.max(state["m"], axis=0, keepdims=True)
                    MB[slot, qt] = jnp.broadcast_to(m, (8, 128))
            return f
        return [mk(int(qt), kt) for qt in qord for kt in range(int(qt) + 1)]

    def p2_steps(g, h, slot, qord, first_seg):
        state = {}
        def mk(qt, kt):
            def f():
                if kt == 0:
                    state["m"] = MB[slot, qt]
                    state["l"] = state["acc"] = None
                s = SB[slot, OFF[qt] + kt * T:OFF[qt] + (kt + 1) * T, :]
                p = jnp.exp2(s.reshape(16, 8, 128) - state["m"][None])
                ps = jnp.sum(p, axis=0)
                pv = dot_nn(VT[g, DH * h:DH * h + DH, kt * T:(kt + 1) * T],
                            p.reshape(T, 128).astype(BF))
                state["l"] = ps if state["l"] is None else state["l"] + ps
                state["acc"] = pv if state["acc"] is None else state["acc"] + pv
                if kt == qt:
                    lt = jnp.sum(state["l"], axis=0, keepdims=True)
                    w = (1.0 - GATE[4 * g + h][0:1, :]) / lt
                    res = state["acc"] * w
                    if not first_seg:
                        res = res + OT[g, DH * h:DH * h + DH, qt * T:(qt + 1) * T]
                    OT[g, DH * h:DH * h + DH, qt * T:(qt + 1) * T] = res
            return f
        return [mk(int(qt), kt) for qt in qord for kt in range(int(qt) + 1)]

    def tr_steps(g):
        def mk(qt):
            def f():
                OB[g, qt * T:(qt + 1) * T, :] = OT[g, :, qt * T:(qt + 1) * T].T.astype(BF)
            return f
        return [mk(qt) for qt in range(NT)]

    def block_a(s):
        for g in range(G):
            for h in range(4):
                a = p2_steps(g, h, h % 2, QORD, s == 0)
                if h < 3:
                    b = p1_steps(g, h + 1, (h + 1) % 2, QORD)
                elif g < G - 1:
                    b = p1_steps(g + 1, 0, 0, QORD)
                elif s < NSEG - 1:
                    b = update_pieces(s)
                else:
                    b = []
                t = tr_steps(g - 1) if (h == 0 and g > 0) else []
                for i in range(10):
                    if i < len(b):
                        b[i]()
                    a[i]()
                    if i < len(t):
                        t[i]()

    def cut(fn):
        lax.fori_loop(0, pl.program_id(0) + 1, lambda i, c: (fn(), c)[1], 0)

    def block_b0(li):
        kp, qp, vp = k_pieces(0), q_pieces(0), v_pieces(0)
        if li == 0:
            for grp in ((0,), (1,), (2, 3), (4, 5, 6, 7)):
                for g in grp:
                    cwk[g].wait()
                for g in grp:
                    kp[g]()
            cwq.wait()
            interleave(qp[:5])
            cwv.wait()
            interleave(qp[5:], wvt_pieces())
        else:
            interleave(kp + qp)
        interleave(vp, p1_steps(0, 0, 0, "0123"))

    def block_b(li, s):
        kp, qp, vp = k_pieces(s), q_pieces(s), v_pieces(s)
        for f in tr_steps(G - 1):
            f()
        interleave(o_pieces(s - 1), ln1_pieces(s))
        ln2, rp = ln2_pieces(s - 1), r_pieces(s - 1)
        q4 = len(ln2) // 4
        interleave(kp[:4], ln2[0:q4])
        interleave(kp[4:], ln2[q4:2 * q4])
        rp[0]()
        interleave(qp[:4], ln2[2 * q4:3 * q4])
        rp[1]()
        interleave(qp[4:], ln2[3 * q4:])
        rp[2]()
        interleave(vp[:2])
        rp[3]()
        if li == 1:
            cout[s - 1].start()
        interleave(vp[2:6], retrieve_pieces())
        interleave(vp[6:], p1_steps(0, 0, 0, "0123"))

    def block_t(li):
        s = NSEG - 1
        for f in tr_steps(G - 1):
            f()
        top2_prefix()
        op, ln2 = o_row_pieces(s), ln2_pieces(s, 12, True)
        q4 = len(ln2) // 4
        op[0]()
        interleave([op[1]], ln2[0:q4])
        interleave([op[2]], ln2[q4:2 * q4])
        interleave([op[3]], ln2[2 * q4:3 * q4])
        interleave(ln2[3 * q4:])
        if li == 1:
            cout[s].start()

    def block_f(li):
        if li == 0:
            interleave(ln1_pieces(0))
        t1, t2 = TOP[0], TOP[1]
        k1 = jnp.broadcast_to(jnp.max(t1, axis=0, keepdims=True), (8, 128))
        k2 = jnp.max(jnp.where(t1 == k1, t2, t1), axis=0, keepdims=True)
        k2 = jnp.broadcast_to(k2, (8, 128))
        i1 = jnp.clip(0xFFFF - (k1[0, 0] & 0xFFFF), 0, S - 1)
        i2 = jnp.clip(0xFFFF - (k2[0, 0] & 0xFFFF), 0, S - 1)
        bases = [pl.multiple_of((i >> 4) << 4, 16) for i in (i1, i2)]
        xs = jnp.concatenate([XN2[pl.ds(b, 16), :] for b in bases], axis=0)
        hs = []
        for j in range(NF):
            gg = rb(dot_nn(xs, WG[:, j * T:(j + 1) * T]))
            uu = rb(dot_nn(xs, WU[:, j * T:(j + 1) * T]))
            hs.append((rb(gg * jax.nn.sigmoid(gg)) * uu).astype(BF))
        hh = jnp.concatenate(hs, axis=1)
        ys = [rb(dot_nn(hh, WD[n])) for n in range(D // T)]
        row16 = lax.broadcasted_iota(I32, (16, D), 0)
        ds = []
        for j, (i, base, kk) in enumerate(zip((i1, i2), bases, (k1, k2))):
            u = kk & I32(-65536)
            mv = pltpu.bitcast(u ^ ((u >> 31) & 0x7FFF0000), F32)
            rs = rb(jax.nn.sigmoid(mv))
            rs = jnp.concatenate([rs, rs], axis=0)
            upd = jnp.concatenate([rb(yn[16 * j:16 * j + 16, :] * rs) for yn in ys], axis=1)
            ds.append(jnp.where(row16 == i - base, upd, 0.0))
        same = bases[0] == bases[1]
        ds = [ds[0] + jnp.where(same, ds[1], 0.0), ds[1] + jnp.where(same, ds[0], 0.0)]
        nbs = [rb(XN2[pl.ds(base, 16), :].astype(F32) + d) for base, d in zip(bases, ds)]
        xos = [(XM[pl.ds(base, 16), :].astype(F32) + nb).astype(BF) for base, nb in zip(bases, nbs)]
        if li == 1:
            cout[NSEG - 1].wait()
        for base, nb, xo in zip(bases, nbs, xos):
            XN2[pl.ds(base, 16), :] = nb.astype(BF)
            X[pl.ds(base, 16), :] = xo
            if li == 0:
                XN[pl.ds(base, 16), :] = layernorm(xo.astype(F32)).astype(BF)
        return bases

    l1 = ln1_pieces(0, chain=False)
    n = len(l1) // NT
    for c in range(NT):
        cx0[c].wait()
        for f in l1[c * n:(c + 1) * n]:
            f()
    for li in range(2):
        for s in range(NSEG):
            if s == 0:
                block_b0(li)
            else:
                block_b(li, s)

            def attn(li=li, s=s):
                block_a(s)
                if li == 0 and s == 0:
                    for c in cx + [cwo]:
                        c.wait()
                    for c in cffn:
                        c.start()
                if li == 0 and s == NSEG - 1:
                    for c in cffn:
                        c.wait()
                if li == 1 and s == NSEG - 1:
                    for c in cout[:NSEG - 1]:
                        c.wait()
            cut(attn)
        block_t(li)
        bases = block_f(li)
    p0 = cp(X.at[pl.ds(bases[0], 16), :], out_hbm.at[pl.ds(bases[0], 16), :], 32)
    p1 = cp(X.at[pl.ds(bases[1], 16), :], out_hbm.at[pl.ds(bases[1], 16), :], 33)
    p0.start()

    @pl.when(bases[1] != bases[0])
    def _():
        p1.start()
        p1.wait()

    p0.wait()


@jax.jit
def pallas_interleave_layers__memory_aug_infini_attn__moe_arch_mod__prompt_kernel(
    A_x, A_wq, A_wk, A_wv, A_wo, A_beta, B_x, B_w_r, B_w_gate, B_w_up, B_w_down):
    del B_x
    any_spec = pl.BlockSpec(memory_space=pl.ANY)
    vm = pltpu.VMEM
    blk = vm((G, L, 128), BF)
    out = pl.pallas_call(
        kernel,
        out_shape=jax.ShapeDtypeStruct((S, D), BF),
        grid=(1,),
        in_specs=[any_spec, any_spec, any_spec, any_spec, any_spec,
                  pl.BlockSpec((1, H), lambda i: (0, 0)), pl.BlockSpec((8, 128), lambda i: (0, 0)),
                  any_spec, any_spec, any_spec],
        out_specs=any_spec,
        scratch_shapes=[
            vm((S, D), BF), vm((S, D), BF), vm((S, D), BF), vm((S, D), BF),
            vm((D, D), BF), vm((D, D), BF), vm((D, D), BF), vm((D, D), BF), vm((D, D), BF),
            vm((D, F), BF), vm((D, F), BF), vm((D // T, F, T), BF),
            blk, blk, blk, blk, vm((G, 128, L), BF),
            vm((2, 1280, 128), F32), vm((2, NT, 8, 128), F32),
            vm((G, 128, L), F32), blk,
            vm((G, 128, 128), F32), vm((G, 8, 128), F32), vm((G, 144, 128), BF),
            vm((H, 8, 128), F32), vm((8, D), F32), vm((16, D), BF), vm((2, 8, 128), I32),
            vm((16, 128), I32),
            pltpu.SemaphoreType.DMA((34,)),
        ],
        compiler_params=pltpu.CompilerParams(vmem_limit_bytes=110 * 1024 * 1024),
        name="fused",
    )(A_x.reshape(S, D), A_wq, A_wk, A_wv, A_wo, A_beta.reshape(1, H), B_w_r.reshape(8, 128),
      B_w_gate, B_w_up, B_w_down)
    return out.reshape(1, S, D)
```

```python
import jax
import jax.numpy as jnp
import numpy as np
from jax import lax
import jax.experimental.pallas as pl
import jax.experimental.pallas.tpu as pltpu

S, D, F = 2048, 1024, 3584
H, DH = 32, 32
NSEG, L = 4, 512
G, T = 8, 128
NT = L // T
NF = F // T
OFF = (0, 128, 384, 768)
NEG = -1e30
EPS = 1e-5
QSCALE = float(DH ** -0.5 * np.log2(np.e))
BF = jnp.bfloat16
F32 = jnp.float32
I32 = jnp.int32
IMIN = -2 ** 31
LNR = 32
QORD = "1302"


def dot_nt(a, b):
    return lax.dot_general(a, b, (((1,), (1,)), ((), ())), preferred_element_type=F32)


def dot_nn(a, b):
    return lax.dot_general(a, b, (((1,), (0,)), ((), ())), preferred_element_type=F32)


def rb(x):
    return x.astype(BF).astype(F32)


def layernorm(x, chain=None):
    m = jnp.sum(x, axis=-1, keepdims=True) * (1.0 / D)
    if chain is not None and chain["tok"] is not None:
        m = jnp.where(chain["never"], chain["tok"], m)
    c = x - m
    v = jnp.sum(c * c, axis=-1, keepdims=True) * (1.0 / D)
    a = rb(rb(v) + EPS)
    y = lax.rsqrt(a)
    s = rb(a * y)
    y = y * (2.0 - s * y)
    if chain is not None:
        chain["tok"] = y
    return c * y


def phi(t):
    return jnp.where(t > 0, t + 1.0, jnp.exp(t))


def head_mask(x, h):
    u = pltpu.bitcast(x, jnp.uint32)
    lane = lax.broadcasted_iota(I32, u.shape, 1)
    u = jnp.where((lane >= DH * h) & (lane < DH * h + DH), u, jnp.uint32(0))
    return pltpu.bitcast(u, BF)


def score_key(sc, tok):
    u = pltpu.bitcast(sc, I32)
    return (u ^ ((u >> 31) & 0x7FFF0000)) | (0xFFFF - tok)


def interleave(main, *bgs):
    done = [0] * len(bgs)
    n = len(main)
    for i, piece in enumerate(main):
        piece()
        for bi, b in enumerate(bgs):
            upto = (i + 1) * len(b) // n
            while done[bi] < upto:
                b[done[bi]]()
                done[bi] += 1


def kernel(x_hbm, wq_hbm, wk_hbm, wv_hbm, wo_hbm, beta_hbm, wr_hbm, wg_hbm, wu_hbm, wd_hbm,
           out_hbm,
           X, XM, XN2, XN, WQ, WK, WV, WVT, WO, WG, WU, WD,
           QS, KK, PQ, PK, VT, SB, MB, OT, OB, MT, ZZ, AMEM, GATE, WR, WRB, TOP, RALL, beta_ref, wr_ref, sems):

    def cp(src, dst, i):
        return pltpu.make_async_copy(src, dst, sems.at[i])
    cx0 = [cp(x_hbm.at[pl.ds(c * T, T), :], X.at[pl.ds(c * T, T), :], c) for c in range(NT)]
    cx = [cp(x_hbm.at[pl.ds(s * L, L), :], X.at[pl.ds(s * L, L), :], 3 + s) for s in range(1, NSEG)]
    cwk = [cp(wk_hbm.at[:, pl.ds(g * T, T)], WK.at[:, pl.ds(g * T, T)], 7 + g) for g in range(G)]
    cwq, cwv, cwo = cp(wq_hbm, WQ, 15), cp(wv_hbm, WV, 16), cp(wo_hbm, WO, 17)
    cffn = ([cp(wg_hbm, WG, 18), cp(wu_hbm, WU, 19)]
            + [cp(wd_hbm.at[:, pl.ds(j * T, T)], WD.at[j], 20 + j) for j in range(D // T)])
    cout = [cp(X.at[pl.ds(s * L, L), :], out_hbm.at[pl.ds(s * L, L), :], 28 + s) for s in range(NSEG)]

    csmall = [cp(beta_hbm, beta_ref, 34), cp(wr_hbm, wr_ref, 35)]
    for c in cx0[:1] + csmall + cx0[1:] + cwk + [cwq, cwv, cx[0], cwo, cx[1], cx[2]]:
        c.start()
    for c in csmall:
        c.wait()

    gate = jax.nn.sigmoid(beta_ref[...].astype(F32))
    for j in range(H):
        GATE[j] = jnp.broadcast_to(gate[:, j:j + 1], (8, 128))
    wr8 = wr_ref[...].astype(F32)
    WR[...] = jnp.concatenate(
        [jnp.broadcast_to(wr8[c:c + 1, :], (8, 128)) for c in range(8)], axis=1)
    WRB[...] = jnp.concatenate(
        [jnp.broadcast_to(wr8[c:c + 1, :], (16, 128)) for c in range(8)], axis=1).astype(BF)
    RALL[...] = jnp.full(RALL.shape, IMIN, I32)

    rowT = lax.broadcasted_iota(I32, (T, T), 0)
    colT = lax.broadcasted_iota(I32, (T, T), 1)
    never = GATE[0][0:1, 0:1] < -1.0

    def new_chain():
        return dict(never=never, tok=None)

    def ln1_pieces(s, chain=True):
        ch = new_chain() if chain else None
        def mk(r):
            def f():
                rr = slice(s * L + r * LNR, s * L + (r + 1) * LNR)
                XN[rr, :] = layernorm(X[rr, :].astype(F32), ch).astype(BF)
            return f
        return [mk(r) for r in range(L // LNR)]

    def ln2_pieces(s, chain_upto=L // LNR, route=False):
        ch = new_chain()
        nrg = LNR // 8
        def mk(r):
            def f():
                if r >= chain_upto:
                    ch["tok"] = None
                r0 = s * L + r * LNR
                rr = slice(r0, r0 + LNR)
                xm = XM[rr, :].astype(F32)
                xn2 = layernorm(xm, ch).astype(BF)
                XN2[rr, :] = xn2
                xf = xn2.astype(F32)
                X[rr, :] = (xm + xf).astype(BF)
                if route:
                    prod = xf.reshape(nrg, 8, D) * WR[...][None]
                    sc = rb(jnp.sum(prod, axis=-1, keepdims=True))
                    sc = jnp.broadcast_to(sc, (nrg, 8, 128)).reshape(LNR, 128)
                    key = score_key(sc, r0 + lax.broadcasted_iota(I32, (LNR, 128), 0))
                    t1, t2 = TOP[0], TOP[1]
                    for j in range(nrg):
                        kj = key[8 * j:8 * j + 8]
                        t2 = jnp.maximum(t2, jnp.minimum(t1, kj))
                        t1 = jnp.maximum(t1, kj)
                    TOP[0] = t1
                    TOP[1] = t2
            return f
        return [mk(r) for r in range(L // LNR)]

    def r_pieces(s):
        def mk(c):
            def f():
                r0 = s * L + c * T
                rr = dot_nt(WRB[...], XN2[r0:r0 + T, :])
                key = score_key(rb(rr[0:8, :]), r0 + lax.broadcasted_iota(I32, (8, 128), 1))
                RALL[s * NT + c:s * NT + c + 1, :] = key[0:1, :]
            return f
        return [mk(c) for c in range(NT)]

    def top2_prefix():
        k = RALL[...]
        k1 = jnp.max(jnp.maximum(k[0:8], k[8:16]), axis=(0, 1), keepdims=True)
        k = jnp.where(k == k1, IMIN, k)
        k2 = jnp.max(jnp.maximum(k[0:8], k[8:16]), axis=(0, 1), keepdims=True)
        TOP[0] = jnp.broadcast_to(k1, (8, 128))
        TOP[1] = jnp.broadcast_to(k2, (8, 128))

    def k_pieces(s):
        rr = slice(s * L, (s + 1) * L)
        def mk(g):
            def f():
                k = dot_nn(XN[rr, :], WK[:, g * T:(g + 1) * T])
                KK[g] = k.astype(BF)
                if s < NSEG - 1:
                    pk = phi(k)
                    PK[g] = pk.astype(BF)
                    z = jnp.sum(pk.reshape(L // 8, 8, 128), axis=0)
                    z = jnp.broadcast_to(jnp.sum(z, axis=0, keepdims=True), (8, 128))
                    ZZ[g] = z if s == 0 else ZZ[g] + z
            return f
        return [mk(g) for g in range(G)]

    def q_pieces(s):
        rr = slice(s * L, (s + 1) * L)
        def mk(g):
            def f():
                q = dot_nn(XN[rr, :], WQ[:, g * T:(g + 1) * T])
                QS[g] = (q * QSCALE).astype(BF)
                if s > 0:
                    PQ[g] = phi(q).astype(BF)
            return f
        return [mk(g) for g in range(G)]

    def v_pieces(s):
        def mk(hf, c):
            def f():
                vt = dot_nt(WVT[hf * L:(hf + 1) * L, :], XN[s * L + c * T:s * L + (c + 1) * T, :])
                for gg in range(4):
                    VT[hf * 4 + gg, :, c * T:(c + 1) * T] = vt[gg * T:(gg + 1) * T, :].astype(BF)
            return f
        return [mk(hf, c) for hf in range(2) for c in range(NT)]

    def o_pieces(s):
        rr = slice(s * L, (s + 1) * L)
        def mk(j):
            def f():
                o = jnp.concatenate([OB[g] for g in range(G)], axis=1)
                y = dot_nn(o, WO[:, j * T:(j + 1) * T])
                XM[rr, j * T:(j + 1) * T] = (X[rr, j * T:(j + 1) * T].astype(F32) + rb(y)).astype(BF)
            return f
        return [mk(j) for j in range(G)]

    def o_row_pieces(s):
        def mk(c):
            def f():
                rr = slice(s * L + c * T, s * L + (c + 1) * T)
                o = jnp.concatenate([OB[g, c * T:(c + 1) * T, :] for g in range(G)], axis=1)
                y = dot_nn(o, WO[...])
                XM[rr, :] = (X[rr, :].astype(F32) + rb(y)).astype(BF)
            return f
        return [mk(c) for c in range(NT)]

    def wvt_pieces():
        def mk(i):
            def f():
                for j in range(D // T):
                    WVT[j * T:(j + 1) * T, i * T:(i + 1) * T] = (
                        WV[i * T:(i + 1) * T, j * T:(j + 1) * T].astype(F32).T.astype(BF))
            return f
        return [mk(i) for i in range(D // T)]

    def retrieve_pieces():
        def mk(g):
            def f():
                r = dot_nt(AMEM[g], PQ[g])
                for h in range(4):
                    den = r[128 + 4 * h:129 + 4 * h, :] + 1e-6
                    OT[g, DH * h:DH * h + DH, :] = (
                        r[DH * h:DH * h + DH, :] * (GATE[4 * g + h][0:1, 0:1] / den))
            return f
        return [mk(g) for g in range(G)]

    def update_pieces(s):
        def mk(g):
            def f():
                upd = dot_nn(VT[g], PK[g])
                rr = lax.broadcasted_iota(I32, (128, 128), 0) // DH
                cc = lax.broadcasted_iota(I32, (128, 128), 1) // DH
                upd = jnp.where(rr == cc, upd, 0.0)
                mt = upd if s == 0 else MT[g] + upd
                if s < NSEG - 2:
                    MT[g] = mt
                AMEM[g, 0:128, :] = mt.astype(BF)
                zr = lax.broadcasted_iota(I32, (16, 128), 0) // 4
                zc = lax.broadcasted_iota(I32, (16, 128), 1) // DH
                z = ZZ[g]
                AMEM[g, 128:144, :] = jnp.where(zr == zc, jnp.concatenate([z, z], axis=0), 0.0).astype(BF)
            return f
        return [mk(g) for g in range(G)]

    def p1_steps(g, h, slot, qord):
        state = {}
        def mk(qt, kt):
            def f():
                if kt == 0:
                    state["qm"] = head_mask(QS[g, qt * T:(qt + 1) * T, :], h)
                    state["m"] = None
                s = dot_nt(KK[g, kt * T:(kt + 1) * T, :], state["qm"])
                if kt == qt:
                    s = jnp.where(rowT <= colT, s, NEG)
                SB[slot, OFF[qt] + kt * T:OFF[qt] + (kt + 1) * T, :] = s
                mt = jnp.max(s.reshape(16, 8, 128), axis=0)
                state["m"] = mt if state["m"] is None else jnp.maximum(state["m"], mt)
                if kt == qt:
                    m = jnp.max(state["m"], axis=0, keepdims=True)
                    MB[slot, qt] = jnp.broadcast_to(m, (8, 128))
            return f
        return [mk(int(qt), kt) for qt in qord for kt in range(int(qt) + 1)]

    def p2_steps(g, h, slot, qord, first_seg):
        state = {}
        def mk(qt, kt):
            def f():
                if kt == 0:
                    state["m"] = MB[slot, qt]
                    state["l"] = state["acc"] = None
                s = SB[slot, OFF[qt] + kt * T:OFF[qt] + (kt + 1) * T, :]
                p = jnp.exp2(s.reshape(16, 8, 128) - state["m"][None])
                ps = jnp.sum(p, axis=0)
                pv = dot_nn(VT[g, DH * h:DH * h + DH, kt * T:(kt + 1) * T],
                            p.reshape(T, 128).astype(BF))
                state["l"] = ps if state["l"] is None else state["l"] + ps
                state["acc"] = pv if state["acc"] is None else state["acc"] + pv
                if kt == qt:
                    lt = jnp.sum(state["l"], axis=0, keepdims=True)
                    w = (1.0 - GATE[4 * g + h][0:1, :]) / lt
                    res = state["acc"] * w
                    if not first_seg:
                        res = res + OT[g, DH * h:DH * h + DH, qt * T:(qt + 1) * T]
                    OT[g, DH * h:DH * h + DH, qt * T:(qt + 1) * T] = res
            return f
        return [mk(int(qt), kt) for qt in qord for kt in range(int(qt) + 1)]

    def tr_steps(g):
        def mk(qt):
            def f():
                OB[g, qt * T:(qt + 1) * T, :] = OT[g, :, qt * T:(qt + 1) * T].T.astype(BF)
            return f
        return [mk(qt) for qt in range(NT)]

    def block_a(s):
        for g in range(G):
            for h in range(4):
                a = p2_steps(g, h, h % 2, QORD, s == 0)
                if h < 3:
                    b = p1_steps(g, h + 1, (h + 1) % 2, QORD)
                elif g < G - 1:
                    b = p1_steps(g + 1, 0, 0, QORD)
                elif s < NSEG - 1:
                    b = update_pieces(s)
                else:
                    b = []
                t = tr_steps(g - 1) if (h == 0 and g > 0) else []
                for i in range(10):
                    if i < len(b):
                        b[i]()
                    a[i]()
                    if i < len(t):
                        t[i]()

    def cut(fn):
        lax.fori_loop(0, pl.program_id(0) + 1, lambda i, c: (fn(), c)[1], 0)

    def block_b0(li):
        kp, qp, vp = k_pieces(0), q_pieces(0), v_pieces(0)
        if li == 0:
            for grp in ((0,), (1,), (2, 3), (4, 5, 6, 7)):
                for g in grp:
                    cwk[g].wait()
                for g in grp:
                    kp[g]()
            cwq.wait()
            interleave(qp[:5])
            cwv.wait()
            interleave(qp[5:], wvt_pieces())
        else:
            interleave(kp + qp)
        interleave(vp, p1_steps(0, 0, 0, "0123"))

    def block_b(li, s):
        kp, qp, vp = k_pieces(s), q_pieces(s), v_pieces(s)
        for f in tr_steps(G - 1):
            f()
        interleave(o_pieces(s - 1), ln1_pieces(s))
        ln2, rp = ln2_pieces(s - 1), r_pieces(s - 1)
        q4 = len(ln2) // 4
        interleave(kp[:4], ln2[0:q4])
        interleave(kp[4:], ln2[q4:2 * q4])
        rp[0]()
        interleave(qp[:4], ln2[2 * q4:3 * q4])
        rp[1]()
        interleave(qp[4:], ln2[3 * q4:])
        rp[2]()
        interleave(vp[:2])
        rp[3]()
        if li == 1:
            cout[s - 1].start()
        interleave(vp[2:6], retrieve_pieces())
        interleave(vp[6:], p1_steps(0, 0, 0, "0123"))

    def block_t(li):
        s = NSEG - 1
        for f in tr_steps(G - 1):
            f()
        top2_prefix()
        op, ln2 = o_row_pieces(s), ln2_pieces(s, 12, True)
        q4 = len(ln2) // 4
        op[0]()
        interleave([op[1]], ln2[0:q4])
        interleave([op[2]], ln2[q4:2 * q4])
        interleave([op[3]], ln2[2 * q4:3 * q4])
        interleave(ln2[3 * q4:])
        if li == 1:
            cout[s].start()

    def block_f(li):
        if li == 0:
            interleave(ln1_pieces(0))
        t1, t2 = TOP[0], TOP[1]
        k1 = jnp.broadcast_to(jnp.max(t1, axis=0, keepdims=True), (8, 128))
        k2 = jnp.max(jnp.where(t1 == k1, t2, t1), axis=0, keepdims=True)
        k2 = jnp.broadcast_to(k2, (8, 128))
        i1 = jnp.clip(0xFFFF - (k1[0, 0] & 0xFFFF), 0, S - 1)
        i2 = jnp.clip(0xFFFF - (k2[0, 0] & 0xFFFF), 0, S - 1)
        bases = [pl.multiple_of((i >> 4) << 4, 16) for i in (i1, i2)]
        xs = jnp.concatenate([XN2[pl.ds(b, 16), :] for b in bases], axis=0)
        hs = []
        for j in range(NF):
            gg = rb(dot_nn(xs, WG[:, j * T:(j + 1) * T]))
            uu = rb(dot_nn(xs, WU[:, j * T:(j + 1) * T]))
            hs.append((rb(gg * jax.nn.sigmoid(gg)) * uu).astype(BF))
        hh = jnp.concatenate(hs, axis=1)
        ys = [rb(dot_nn(hh, WD[n])) for n in range(D // T)]
        row16 = lax.broadcasted_iota(I32, (16, D), 0)
        ds = []
        for j, (i, base, kk) in enumerate(zip((i1, i2), bases, (k1, k2))):
            u = kk & I32(-65536)
            mv = pltpu.bitcast(u ^ ((u >> 31) & 0x7FFF0000), F32)
            rs = rb(jax.nn.sigmoid(mv))
            rs = jnp.concatenate([rs, rs], axis=0)
            upd = jnp.concatenate([rb(yn[16 * j:16 * j + 16, :] * rs) for yn in ys], axis=1)
            ds.append(jnp.where(row16 == i - base, upd, 0.0))
        same = bases[0] == bases[1]
        ds = [ds[0] + jnp.where(same, ds[1], 0.0), ds[1] + jnp.where(same, ds[0], 0.0)]
        nbs = [rb(XN2[pl.ds(base, 16), :].astype(F32) + d) for base, d in zip(bases, ds)]
        xos = [(XM[pl.ds(base, 16), :].astype(F32) + nb).astype(BF) for base, nb in zip(bases, nbs)]
        if li == 1:
            cout[NSEG - 1].wait()
        for base, nb, xo in zip(bases, nbs, xos):
            XN2[pl.ds(base, 16), :] = nb.astype(BF)
            X[pl.ds(base, 16), :] = xo
            if li == 0:
                XN[pl.ds(base, 16), :] = layernorm(xo.astype(F32)).astype(BF)
        return bases

    l1 = ln1_pieces(0, chain=False)
    n = len(l1) // NT
    for c in range(NT):
        cx0[c].wait()
        for f in l1[c * n:(c + 1) * n]:
            f()
    for li in range(2):
        for s in range(NSEG):
            if s == 0:
                block_b0(li)
            else:
                block_b(li, s)

            def attn(li=li, s=s):
                block_a(s)
                if li == 0 and s == 0:
                    for c in cx + [cwo]:
                        c.wait()
                    for c in cffn:
                        c.start()
                if li == 0 and s == NSEG - 1:
                    for c in cffn:
                        c.wait()
                if li == 1 and s == NSEG - 1:
                    for c in cout[:NSEG - 1]:
                        c.wait()
            cut(attn)
        block_t(li)
        bases = block_f(li)
    p0 = cp(X.at[pl.ds(bases[0], 16), :], out_hbm.at[pl.ds(bases[0], 16), :], 32)
    p1 = cp(X.at[pl.ds(bases[1], 16), :], out_hbm.at[pl.ds(bases[1], 16), :], 33)
    p0.start()

    @pl.when(bases[1] != bases[0])
    def _():
        p1.start()
        p1.wait()

    p0.wait()


@jax.jit
def pallas_interleave_layers__memory_aug_infini_attn__moe_arch_mod__prompt_kernel(
    A_x, A_wq, A_wk, A_wv, A_wo, A_beta, B_x, B_w_r, B_w_gate, B_w_up, B_w_down):
    del B_x
    any_spec = pl.BlockSpec(memory_space=pl.ANY)
    vm = pltpu.VMEM
    blk = vm((G, L, 128), BF)
    out = pl.pallas_call(
        kernel,
        out_shape=jax.ShapeDtypeStruct((S, D), BF),
        grid=(1,),
        in_specs=[any_spec, any_spec, any_spec, any_spec, any_spec,
                  any_spec, any_spec,
                  any_spec, any_spec, any_spec],
        out_specs=any_spec,
        scratch_shapes=[
            vm((S, D), BF), vm((S, D), BF), vm((S, D), BF), vm((S, D), BF),
            vm((D, D), BF), vm((D, D), BF), vm((D, D), BF), vm((D, D), BF), vm((D, D), BF),
            vm((D, F), BF), vm((D, F), BF), vm((D // T, F, T), BF),
            blk, blk, blk, blk, vm((G, 128, L), BF),
            vm((2, 1280, 128), F32), vm((2, NT, 8, 128), F32),
            vm((G, 128, L), F32), blk,
            vm((G, 128, 128), F32), vm((G, 8, 128), F32), vm((G, 144, 128), BF),
            vm((H, 8, 128), F32), vm((8, D), F32), vm((16, D), BF), vm((2, 8, 128), I32),
            vm((16, 128), I32), vm((1, H), BF), vm((8, 128), BF),
            pltpu.SemaphoreType.DMA((36,)),
        ],
        compiler_params=pltpu.CompilerParams(vmem_limit_bytes=110 * 1024 * 1024),
        name="fused",
    )(A_x.reshape(S, D), A_wq, A_wk, A_wv, A_wo, A_beta.reshape(1, H), B_w_r.reshape(8, 128),
      B_w_gate, B_w_up, B_w_down)
    return out.reshape(1, S, D)
```

```python
import jax
import jax.numpy as jnp
import numpy as np
from jax import lax
import jax.experimental.pallas as pl
import jax.experimental.pallas.tpu as pltpu

S, D, F = 2048, 1024, 3584
H, DH = 32, 32
NSEG, L = 4, 512
G, T = 8, 128
NT = L // T
NF = F // T
OFF = (0, 128, 384, 768)
NEG = -1e30
EPS = 1e-5
QSCALE = float(DH ** -0.5 * np.log2(np.e))
BF = jnp.bfloat16
F32 = jnp.float32
I32 = jnp.int32
IMIN = -2 ** 31
LNR = 32
QORD = "1302"


def dot_nt(a, b):
    return lax.dot_general(a, b, (((1,), (1,)), ((), ())), preferred_element_type=F32)


def dot_nn(a, b):
    return lax.dot_general(a, b, (((1,), (0,)), ((), ())), preferred_element_type=F32)


def rb(x):
    return x.astype(BF).astype(F32)


def layernorm(x, chain=None):
    m = jnp.sum(x, axis=-1, keepdims=True) * (1.0 / D)
    if chain is not None and chain["tok"] is not None:
        m = jnp.where(chain["never"], chain["tok"], m)
    c = x - m
    v = jnp.sum(c * c, axis=-1, keepdims=True) * (1.0 / D)
    a = rb(rb(v) + EPS)
    y = lax.rsqrt(a)
    s = rb(a * y)
    y = y * (2.0 - s * y)
    if chain is not None:
        chain["tok"] = y
    return c * y


def phi(t):
    return jnp.where(t > 0, t + 1.0, jnp.exp(t))


def head_mask(x, h):
    u = pltpu.bitcast(x, jnp.uint32)
    lane = lax.broadcasted_iota(I32, u.shape, 1)
    u = jnp.where((lane >= DH * h) & (lane < DH * h + DH), u, jnp.uint32(0))
    return pltpu.bitcast(u, BF)


def score_key(sc, tok):
    u = pltpu.bitcast(sc, I32)
    return (u ^ ((u >> 31) & 0x7FFF0000)) | (0xFFFF - tok)


def interleave(main, *bgs):
    done = [0] * len(bgs)
    n = len(main)
    for i, piece in enumerate(main):
        piece()
        for bi, b in enumerate(bgs):
            upto = (i + 1) * len(b) // n
            while done[bi] < upto:
                b[done[bi]]()
                done[bi] += 1


def kernel(x_hbm, wq_hbm, wk_hbm, wv_hbm, wo_hbm, beta_hbm, wr_hbm, wg_hbm, wu_hbm, wd_hbm,
           out_hbm,
           X, XM, XN2, XN, WQ, WK, WV, WVT, WO, WG, WU, WD,
           QS, KK, PQ, PK, VT, SB, MB, OT, OB, MT, ZZ, AMEM, GATE, WR, WRB, TOP, RALL, beta_ref, wr_ref, sems):

    def cp(src, dst, i):
        return pltpu.make_async_copy(src, dst, sems.at[i])
    cx0 = [cp(x_hbm.at[pl.ds(c * T, T), :], X.at[pl.ds(c * T, T), :], c) for c in range(NT)]
    cx = [cp(x_hbm.at[pl.ds(s * L, L), :], X.at[pl.ds(s * L, L), :], 3 + s) for s in range(1, NSEG)]
    cwk = [cp(wk_hbm.at[:, pl.ds(g * T, T)], WK.at[:, pl.ds(g * T, T)], 7 + g) for g in range(G)]
    cwq, cwv, cwo = cp(wq_hbm, WQ, 15), cp(wv_hbm, WV, 16), cp(wo_hbm, WO, 17)
    cffn = ([cp(wg_hbm, WG, 18), cp(wu_hbm, WU, 19)]
            + [cp(wd_hbm.at[:, pl.ds(j * T, T)], WD.at[j], 20 + j) for j in range(D // T)])
    cout = [cp(X.at[pl.ds(s * L, L), :], out_hbm.at[pl.ds(s * L, L), :], 28 + s) for s in range(NSEG)]

    csmall = [cp(beta_hbm, beta_ref, 34), cp(wr_hbm, wr_ref, 35)]
    for c in csmall + cx0 + cwk + [cwq, cwv, cx[0], cwo, cx[1], cx[2]]:
        c.start()

    def init_pieces():
        def gates(j0):
            def f():
                gate = jax.nn.sigmoid(beta_ref[...].astype(F32))
                for j in range(j0, j0 + 8):
                    GATE[j] = jnp.broadcast_to(gate[:, j:j + 1], (8, 128))
            return f
        def router():
            wr8 = wr_ref[...].astype(F32)
            WR[...] = jnp.concatenate(
                [jnp.broadcast_to(wr8[c:c + 1, :], (8, 128)) for c in range(8)], axis=1)
            WRB[...] = jnp.concatenate(
                [jnp.broadcast_to(wr8[c:c + 1, :], (16, 128)) for c in range(8)], axis=1).astype(BF)
            RALL[...] = jnp.full(RALL.shape, IMIN, I32)
        return [gates(j0) for j0 in range(0, H, 8)] + [router]

    rowT = lax.broadcasted_iota(I32, (T, T), 0)
    colT = lax.broadcasted_iota(I32, (T, T), 1)

    def new_chain():
        return dict(never=GATE[0][0:1, 0:1] < -1.0, tok=None)

    def ln1_pieces(s, chain=True):
        ch = new_chain() if chain else None
        def mk(r):
            def f():
                rr = slice(s * L + r * LNR, s * L + (r + 1) * LNR)
                XN[rr, :] = layernorm(X[rr, :].astype(F32), ch).astype(BF)
            return f
        return [mk(r) for r in range(L // LNR)]

    def ln2_pieces(s, chain_upto=L // LNR, route=False):
        ch = new_chain()
        nrg = LNR // 8
        def mk(r):
            def f():
                if r >= chain_upto:
                    ch["tok"] = None
                r0 = s * L + r * LNR
                rr = slice(r0, r0 + LNR)
                xm = XM[rr, :].astype(F32)
                xn2 = layernorm(xm, ch).astype(BF)
                XN2[rr, :] = xn2
                xf = xn2.astype(F32)
                X[rr, :] = (xm + xf).astype(BF)
                if route:
                    prod = xf.reshape(nrg, 8, D) * WR[...][None]
                    sc = rb(jnp.sum(prod, axis=-1, keepdims=True))
                    sc = jnp.broadcast_to(sc, (nrg, 8, 128)).reshape(LNR, 128)
                    key = score_key(sc, r0 + lax.broadcasted_iota(I32, (LNR, 128), 0))
                    t1, t2 = TOP[0], TOP[1]
                    for j in range(nrg):
                        kj = key[8 * j:8 * j + 8]
                        t2 = jnp.maximum(t2, jnp.minimum(t1, kj))
                        t1 = jnp.maximum(t1, kj)
                    TOP[0] = t1
                    TOP[1] = t2
            return f
        return [mk(r) for r in range(L // LNR)]

    def r_pieces(s):
        def mk(c):
            def f():
                r0 = s * L + c * T
                rr = dot_nt(WRB[...], XN2[r0:r0 + T, :])
                key = score_key(rb(rr[0:8, :]), r0 + lax.broadcasted_iota(I32, (8, 128), 1))
                RALL[s * NT + c:s * NT + c + 1, :] = key[0:1, :]
            return f
        return [mk(c) for c in range(NT)]

    def top2_prefix():
        k = RALL[...]
        k1 = jnp.max(jnp.maximum(k[0:8], k[8:16]), axis=(0, 1), keepdims=True)
        k = jnp.where(k == k1, IMIN, k)
        k2 = jnp.max(jnp.maximum(k[0:8], k[8:16]), axis=(0, 1), keepdims=True)
        TOP[0] = jnp.broadcast_to(k1, (8, 128))
        TOP[1] = jnp.broadcast_to(k2, (8, 128))

    def k_pieces(s):
        rr = slice(s * L, (s + 1) * L)
        def mk(g):
            def f():
                k = dot_nn(XN[rr, :], WK[:, g * T:(g + 1) * T])
                KK[g] = k.astype(BF)
                if s < NSEG - 1:
                    pk = phi(k)
                    PK[g] = pk.astype(BF)
                    z = jnp.sum(pk.reshape(L // 8, 8, 128), axis=0)
                    z = jnp.broadcast_to(jnp.sum(z, axis=0, keepdims=True), (8, 128))
                    ZZ[g] = z if s == 0 else ZZ[g] + z
            return f
        return [mk(g) for g in range(G)]

    def q_pieces(s):
        rr = slice(s * L, (s + 1) * L)
        def mk(g):
            def f():
                q = dot_nn(XN[rr, :], WQ[:, g * T:(g + 1) * T])
                QS[g] = (q * QSCALE).astype(BF)
                if s > 0:
                    PQ[g] = phi(q).astype(BF)
            return f
        return [mk(g) for g in range(G)]

    def v_pieces(s):
        def mk(hf, c):
            def f():
                vt = dot_nt(WVT[hf * L:(hf + 1) * L, :], XN[s * L + c * T:s * L + (c + 1) * T, :])
                for gg in range(4):
                    VT[hf * 4 + gg, :, c * T:(c + 1) * T] = vt[gg * T:(gg + 1) * T, :].astype(BF)
            return f
        return [mk(hf, c) for hf in range(2) for c in range(NT)]

    def o_pieces(s):
        rr = slice(s * L, (s + 1) * L)
        def mk(j):
            def f():
                o = jnp.concatenate([OB[g] for g in range(G)], axis=1)
                y = dot_nn(o, WO[:, j * T:(j + 1) * T])
                XM[rr, j * T:(j + 1) * T] = (X[rr, j * T:(j + 1) * T].astype(F32) + rb(y)).astype(BF)
            return f
        return [mk(j) for j in range(G)]

    def o_row_pieces(s):
        def mk(c):
            def f():
                rr = slice(s * L + c * T, s * L + (c + 1) * T)
                o = jnp.concatenate([OB[g, c * T:(c + 1) * T, :] for g in range(G)], axis=1)
                y = dot_nn(o, WO[...])
                XM[rr, :] = (X[rr, :].astype(F32) + rb(y)).astype(BF)
            return f
        return [mk(c) for c in range(NT)]

    def wvt_pieces():
        def mk(i):
            def f():
                for j in range(D // T):
                    WVT[j * T:(j + 1) * T, i * T:(i + 1) * T] = (
                        WV[i * T:(i + 1) * T, j * T:(j + 1) * T].astype(F32).T.astype(BF))
            return f
        return [mk(i) for i in range(D // T)]

    def retrieve_pieces():
        def mk(g):
            def f():
                r = dot_nt(AMEM[g], PQ[g])
                for h in range(4):
                    den = r[128 + 4 * h:129 + 4 * h, :] + 1e-6
                    OT[g, DH * h:DH * h + DH, :] = (
                        r[DH * h:DH * h + DH, :] * (GATE[4 * g + h][0:1, 0:1] / den))
            return f
        return [mk(g) for g in range(G)]

    def update_pieces(s):
        def mk(g):
            def f():
                upd = dot_nn(VT[g], PK[g])
                rr = lax.broadcasted_iota(I32, (128, 128), 0) // DH
                cc = lax.broadcasted_iota(I32, (128, 128), 1) // DH
                upd = jnp.where(rr == cc, upd, 0.0)
                mt = upd if s == 0 else MT[g] + upd
                if s < NSEG - 2:
                    MT[g] = mt
                AMEM[g, 0:128, :] = mt.astype(BF)
                zr = lax.broadcasted_iota(I32, (16, 128), 0) // 4
                zc = lax.broadcasted_iota(I32, (16, 128), 1) // DH
                z = ZZ[g]
                AMEM[g, 128:144, :] = jnp.where(zr == zc, jnp.concatenate([z, z], axis=0), 0.0).astype(BF)
            return f
        return [mk(g) for g in range(G)]

    def p1_steps(g, h, slot, qord):
        state = {}
        def mk(qt, kt):
            def f():
                if kt == 0:
                    state["qm"] = head_mask(QS[g, qt * T:(qt + 1) * T, :], h)
                    state["m"] = None
                s = dot_nt(KK[g, kt * T:(kt + 1) * T, :], state["qm"])
                if kt == qt:
                    s = jnp.where(rowT <= colT, s, NEG)
                SB[slot, OFF[qt] + kt * T:OFF[qt] + (kt + 1) * T, :] = s
                mt = jnp.max(s.reshape(16, 8, 128), axis=0)
                state["m"] = mt if state["m"] is None else jnp.maximum(state["m"], mt)
                if kt == qt:
                    m = jnp.max(state["m"], axis=0, keepdims=True)
                    MB[slot, qt] = jnp.broadcast_to(m, (8, 128))
            return f
        return [mk(int(qt), kt) for qt in qord for kt in range(int(qt) + 1)]

    def p2_steps(g, h, slot, qord, first_seg):
        state = {}
        def mk(qt, kt):
            def f():
                if kt == 0:
                    state["m"] = MB[slot, qt]
                    state["l"] = state["acc"] = None
                s = SB[slot, OFF[qt] + kt * T:OFF[qt] + (kt + 1) * T, :]
                p = jnp.exp2(s.reshape(16, 8, 128) - state["m"][None])
                ps = jnp.sum(p, axis=0)
                pv = dot_nn(VT[g, DH * h:DH * h + DH, kt * T:(kt + 1) * T],
                            p.reshape(T, 128).astype(BF))
                state["l"] = ps if state["l"] is None else state["l"] + ps
                state["acc"] = pv if state["acc"] is None else state["acc"] + pv
                if kt == qt:
                    lt = jnp.sum(state["l"], axis=0, keepdims=True)
                    w = (1.0 - GATE[4 * g + h][0:1, :]) / lt
                    res = state["acc"] * w
                    if not first_seg:
                        res = res + OT[g, DH * h:DH * h + DH, qt * T:(qt + 1) * T]
                    OT[g, DH * h:DH * h + DH, qt * T:(qt + 1) * T] = res
            return f
        return [mk(int(qt), kt) for qt in qord for kt in range(int(qt) + 1)]

    def tr_steps(g):
        def mk(qt):
            def f():
                OB[g, qt * T:(qt + 1) * T, :] = OT[g, :, qt * T:(qt + 1) * T].T.astype(BF)
            return f
        return [mk(qt) for qt in range(NT)]

    def block_a(s):
        for g in range(G):
            for h in range(4):
                a = p2_steps(g, h, h % 2, QORD, s == 0)
                if h < 3:
                    b = p1_steps(g, h + 1, (h + 1) % 2, QORD)
                elif g < G - 1:
                    b = p1_steps(g + 1, 0, 0, QORD)
                elif s < NSEG - 1:
                    b = update_pieces(s)
                else:
                    b = []
                t = tr_steps(g - 1) if (h == 0 and g > 0) else []
                for i in range(10):
                    if i < len(b):
                        b[i]()
                    a[i]()
                    if i < len(t):
                        t[i]()

    def cut(fn):
        lax.fori_loop(0, pl.program_id(0) + 1, lambda i, c: (fn(), c)[1], 0)

    def block_b0(li):
        kp, qp, vp = k_pieces(0), q_pieces(0), v_pieces(0)
        if li == 0:
            for grp in ((0,), (1,), (2, 3), (4, 5, 6, 7)):
                for g in grp:
                    cwk[g].wait()
                for g in grp:
                    kp[g]()
            for c in [cwq] + csmall:
                c.wait()
            interleave(qp[:5], init_pieces())
            cwv.wait()
            interleave(qp[5:], wvt_pieces())
        else:
            interleave(kp + qp)
        interleave(vp, p1_steps(0, 0, 0, "0123"))

    def block_b(li, s):
        kp, qp, vp = k_pieces(s), q_pieces(s), v_pieces(s)
        for f in tr_steps(G - 1):
            f()
        interleave(o_pieces(s - 1), ln1_pieces(s))
        ln2, rp = ln2_pieces(s - 1), r_pieces(s - 1)
        q4 = len(ln2) // 4
        interleave(kp[:4], ln2[0:q4])
        interleave(kp[4:], ln2[q4:2 * q4])
        rp[0]()
        interleave(qp[:4], ln2[2 * q4:3 * q4])
        rp[1]()
        interleave(qp[4:], ln2[3 * q4:])
        rp[2]()
        interleave(vp[:2])
        rp[3]()
        if li == 1:
            cout[s - 1].start()
        interleave(vp[2:6], retrieve_pieces())
        interleave(vp[6:], p1_steps(0, 0, 0, "0123"))

    def block_t(li):
        s = NSEG - 1
        for f in tr_steps(G - 1):
            f()
        top2_prefix()
        op, ln2 = o_row_pieces(s), ln2_pieces(s, 12, True)
        q4 = len(ln2) // 4
        op[0]()
        interleave([op[1]], ln2[0:q4])
        interleave([op[2]], ln2[q4:2 * q4])
        interleave([op[3]], ln2[2 * q4:3 * q4])
        interleave(ln2[3 * q4:])
        if li == 1:
            cout[s].start()

    def block_f(li):
        if li == 0:
            interleave(ln1_pieces(0))
        t1, t2 = TOP[0], TOP[1]
        k1 = jnp.broadcast_to(jnp.max(t1, axis=0, keepdims=True), (8, 128))
        k2 = jnp.max(jnp.where(t1 == k1, t2, t1), axis=0, keepdims=True)
        k2 = jnp.broadcast_to(k2, (8, 128))
        i1 = jnp.clip(0xFFFF - (k1[0, 0] & 0xFFFF), 0, S - 1)
        i2 = jnp.clip(0xFFFF - (k2[0, 0] & 0xFFFF), 0, S - 1)
        bases = [pl.multiple_of((i >> 4) << 4, 16) for i in (i1, i2)]
        xs = jnp.concatenate([XN2[pl.ds(b, 16), :] for b in bases], axis=0)
        hs = []
        for j in range(NF):
            gg = rb(dot_nn(xs, WG[:, j * T:(j + 1) * T]))
            uu = rb(dot_nn(xs, WU[:, j * T:(j + 1) * T]))
            hs.append((rb(gg * jax.nn.sigmoid(gg)) * uu).astype(BF))
        hh = jnp.concatenate(hs, axis=1)
        ys = [rb(dot_nn(hh, WD[n])) for n in range(D // T)]
        row16 = lax.broadcasted_iota(I32, (16, D), 0)
        ds = []
        for j, (i, base, kk) in enumerate(zip((i1, i2), bases, (k1, k2))):
            u = kk & I32(-65536)
            mv = pltpu.bitcast(u ^ ((u >> 31) & 0x7FFF0000), F32)
            rs = rb(jax.nn.sigmoid(mv))
            rs = jnp.concatenate([rs, rs], axis=0)
            upd = jnp.concatenate([rb(yn[16 * j:16 * j + 16, :] * rs) for yn in ys], axis=1)
            ds.append(jnp.where(row16 == i - base, upd, 0.0))
        same = bases[0] == bases[1]
        ds = [ds[0] + jnp.where(same, ds[1], 0.0), ds[1] + jnp.where(same, ds[0], 0.0)]
        nbs = [rb(XN2[pl.ds(base, 16), :].astype(F32) + d) for base, d in zip(bases, ds)]
        xos = [(XM[pl.ds(base, 16), :].astype(F32) + nb).astype(BF) for base, nb in zip(bases, nbs)]
        if li == 1:
            cout[NSEG - 1].wait()
        for base, nb, xo in zip(bases, nbs, xos):
            XN2[pl.ds(base, 16), :] = nb.astype(BF)
            X[pl.ds(base, 16), :] = xo
            if li == 0:
                XN[pl.ds(base, 16), :] = layernorm(xo.astype(F32)).astype(BF)
        return bases

    l1 = ln1_pieces(0, chain=False)
    n = len(l1) // NT
    for c in range(NT):
        cx0[c].wait()
        for f in l1[c * n:(c + 1) * n]:
            f()
    for li in range(2):
        for s in range(NSEG):
            if s == 0:
                block_b0(li)
            else:
                block_b(li, s)

            def attn(li=li, s=s):
                block_a(s)
                if li == 0 and s == 0:
                    for c in cx + [cwo]:
                        c.wait()
                    for c in cffn:
                        c.start()
                if li == 0 and s == NSEG - 1:
                    for c in cffn:
                        c.wait()
                if li == 1 and s == NSEG - 1:
                    for c in cout[:NSEG - 1]:
                        c.wait()
            cut(attn)
        block_t(li)
        bases = block_f(li)
    p0 = cp(X.at[pl.ds(bases[0], 16), :], out_hbm.at[pl.ds(bases[0], 16), :], 32)
    p1 = cp(X.at[pl.ds(bases[1], 16), :], out_hbm.at[pl.ds(bases[1], 16), :], 33)
    p0.start()

    @pl.when(bases[1] != bases[0])
    def _():
        p1.start()
        p1.wait()

    p0.wait()


@jax.jit
def pallas_interleave_layers__memory_aug_infini_attn__moe_arch_mod__prompt_kernel(
    A_x, A_wq, A_wk, A_wv, A_wo, A_beta, B_x, B_w_r, B_w_gate, B_w_up, B_w_down):
    del B_x
    any_spec = pl.BlockSpec(memory_space=pl.ANY)
    vm = pltpu.VMEM
    blk = vm((G, L, 128), BF)
    out = pl.pallas_call(
        kernel,
        out_shape=jax.ShapeDtypeStruct((S, D), BF),
        grid=(1,),
        in_specs=[any_spec, any_spec, any_spec, any_spec, any_spec,
                  any_spec, any_spec,
                  any_spec, any_spec, any_spec],
        out_specs=any_spec,
        scratch_shapes=[
            vm((S, D), BF), vm((S, D), BF), vm((S, D), BF), vm((S, D), BF),
            vm((D, D), BF), vm((D, D), BF), vm((D, D), BF), vm((D, D), BF), vm((D, D), BF),
            vm((D, F), BF), vm((D, F), BF), vm((D // T, F, T), BF),
            blk, blk, blk, blk, vm((G, 128, L), BF),
            vm((2, 1280, 128), F32), vm((2, NT, 8, 128), F32),
            vm((G, 128, L), F32), blk,
            vm((G, 128, 128), F32), vm((G, 8, 128), F32), vm((G, 144, 128), BF),
            vm((H, 8, 128), F32), vm((8, D), F32), vm((16, D), BF), vm((2, 8, 128), I32),
            vm((16, 128), I32), vm((1, H), BF), vm((8, 128), BF),
            pltpu.SemaphoreType.DMA((36,)),
        ],
        compiler_params=pltpu.CompilerParams(vmem_limit_bytes=110 * 1024 * 1024),
        name="fused",
    )(A_x.reshape(S, D), A_wq, A_wk, A_wv, A_wo, A_beta.reshape(1, H), B_w_r.reshape(8, 128),
      B_w_gate, B_w_up, B_w_down)
    return out.reshape(1, S, D)
```
